```python
import os as _os
_os.environ.setdefault("JAX_PLATFORMS", "cpu")
import jax
import jax.numpy as jnp

def _softmax(x, axis=-1):
    return jax.nn.softmax(x, axis=axis)
def _gelu(x):
    return jax.nn.gelu(x, approximate=True)
def _silu(x):
    return jax.nn.silu(x)
def _sigmoid(x):
    return jax.nn.sigmoid(x)
def _layernorm(x, axis=-1, eps=1e-5):
    m = jnp.mean(x, axis=axis, keepdims=True)
    v = jnp.var(x, axis=axis, keepdims=True)
    return (x - m) / jnp.sqrt(v + eps)
def _scatter_add(tgt, idx, src, axis=0):
    return tgt.at[idx].add(src)
def _segment_sum(src, seg, n):
    return jax.ops.segment_sum(src, seg, n)
class _Rng:
    def __init__(self, key):
        self._k = key
    def _next(self):
        self._k, sub = jax.random.split(self._k)
        return sub
    def normal(self, shape):
        return jax.random.normal(self._next(), shape, dtype=jnp.bfloat16)
    def randint(self, lo, hi, shape):
        return jax.random.randint(self._next(), shape, lo, hi, dtype=jnp.int32)
    def uniform(self, shape, lo=0.0, hi=1.0):
        return jax.random.uniform(self._next(), shape, jnp.bfloat16, lo, hi)
    def permutation(self, n):
        return jax.random.permutation(self._next(), n)


kernel_name = 'sequential_preLN__spectral_gfnet__glu_gated_bilinear__prompt'

def setup_inputs():
    _rng = _Rng(jax.random.key(int.from_bytes(__import__("os").urandom(4), "little")))
    _w = (lambda a: (lambda t: t.astype(jnp.bfloat16) if jnp.issubdtype(t.dtype, jnp.floating) else t)(jnp.asarray(a)))
    def _A_setup():
        B, S, D = 1, 2048, 448
        Df = D // 2 + 1
        return {
            "x": _w((lambda *s: _rng.normal(s) * 0.05)(B, S, D)),
            "w_r": _w((lambda *s: _rng.normal(s) * 0.2)(S, Df) * 0.02),
            "w_i": _w((lambda *s: _rng.normal(s) * 0.2)(S, Df) * 0.02),
        }
    _A_in = _A_setup()

    def _B_setup():
        B, S, D, F = 1, 2048, 448, 1792
        return {
            "x": _w((lambda *s: _rng.normal(s) * 0.05)(B, S, D)),
            "w_gate": _w((lambda *s: _rng.normal(s) * 0.05)(D, F) * (D ** -0.5)),
            "w_up": _w((lambda *s: _rng.normal(s) * 0.05)(D, F) * (D ** -0.5)),
            "w_down": _w((lambda *s: _rng.normal(s) * 0.05)(F, D) * (F ** -0.5)),
        }
    _B_in = _B_setup()

    return {
        "A_x": _A_in["x"],
        "A_w_r": _A_in["w_r"],
        "A_w_i": _A_in["w_i"],
        "B_x": _B_in["x"],
        "B_w_gate": _B_in["w_gate"],
        "B_w_up": _B_in["w_up"],
        "B_w_down": _B_in["w_down"],
    }

def reference(A_x, A_w_r, A_w_i, B_x, B_w_gate, B_w_up, B_w_down):
    def _A_ref(x, w_r, w_i):
        B, S, D = x.shape
        X = (lambda x, axes=(-2,-1): jnp.fft.rfft2(x.astype(jnp.float32), axes=axes))(x, axes=(-2, -1))
        W = w_r + 1j * w_i
        X = X * W
        y = (lambda x, s, axes=(-2,-1): jnp.fft.irfft2(x, s=s, axes=axes).astype(jnp.bfloat16))(X, (S, D), axes=(-2, -1))
        return y

    def _B_ref(x, w_gate, w_up, w_down):
        g = jnp.einsum("bsd,df->bsf", x, w_gate)
        u = jnp.einsum("bsd,df->bsf", x, w_up)
        h = g * u
        return jnp.einsum("bsf,fd->bsd", h, w_down)

    x = A_x
    h = x + _A_ref(_layernorm(x, axis=-1), A_w_r, A_w_i)
    h2 = h + _B_ref(_layernorm(h, axis=-1), B_w_gate, B_w_up, B_w_down)
    return h2
```

```python
import numpy as np
import jax
import jax.numpy as jnp
from jax import lax
from jax.experimental import pallas as pl
from jax.experimental.pallas import tpu as pltpu

S, D, FF = 2048, 448, 1792
H = D // 2
N1, N2 = 32, 64
PZ = N2 + 1
PW = N1 + 1
BF = jnp.bfloat16
F32 = jnp.float32
U32 = jnp.uint32
EPS = 1e-5


def _consts():
    d = np.arange(H)
    rf = np.zeros((512, 256))
    for m in range(H // 2 + 1):
        ang = -2.0 * np.pi * ((2 * m * d) % D) / D
        rf[2 * m, :H] = np.cos(ang)
        rf[2 * m + 1, :H] = np.sin(ang)
    for m in range(H // 2):
        ang = -2.0 * np.pi * (((2 * m + 1) * d) % D) / D
        rf[256 + 2 * m, :H] = np.cos(ang)
        rf[256 + 2 * m + 1, :H] = np.sin(ang)
    ci = np.zeros((2, H, 256))
    for m in range(H // 2 + 1):
        k = 2 * m
        c = 1.0 if (k == 0 or k == H) else 2.0
        ang = 2.0 * np.pi * ((k * d) % D) / D
        ci[0, :, m] = c * np.cos(ang) / (S * D)
        if k != 0 and k != H:
            ci[0, :, 128 + m] = -c * np.sin(ang) / (S * D)
    for m in range(H // 2):
        k = 2 * m + 1
        ang = 2.0 * np.pi * ((k * d) % D) / D
        ci[1, :, m] = 2.0 * np.cos(ang) / (S * D)
        ci[1, :, 128 + m] = -2.0 * np.sin(ang) / (S * D)
    n1 = np.arange(N1)
    n2 = np.arange(N2)
    ang = -2.0 * np.pi * ((np.outer(n1, n1)) % N1) / N1
    fr, fi = np.cos(ang), np.sin(ang)
    fa = np.zeros((2, 128, 128))
    for mu in range(2):
        o = 64 * mu
        fa[0, o + 0:o + 64:2, o + 0:o + 64:2] = fr
        fa[0, o + 0:o + 64:2, o + 1:o + 64:2] = -fi
        fa[0, o + 1:o + 64:2, o + 0:o + 64:2] = fi
        fa[0, o + 1:o + 64:2, o + 1:o + 64:2] = fr
        fa[1, mu:64:2, o + 0:o + 64:2] = fr
        fa[1, mu:64:2, o + 1:o + 64:2] = fi
        fa[1, 64 + mu:128:2, o + 0:o + 64:2] = -fi
        fa[1, 64 + mu:128:2, o + 1:o + 64:2] = fr
    gf = np.zeros((N1, 128, 128))
    gi = np.zeros((N1, 128, 128))
    for k1 in range(N1):
        ang = -2.0 * np.pi * (np.outer(k1 + N1 * n2, n2) % S) / S
        gr, gim = np.cos(ang), np.sin(ang)
        gf[k1, 0:64, 0::2] = gr
        gf[k1, 0:64, 1::2] = -gim
        gf[k1, 64:128, 0::2] = gim
        gf[k1, 64:128, 1::2] = gr
        gi[k1, 0::2, 0:64] = gr.T
        gi[k1, 0::2, 64:128] = gim.T
        gi[k1, 1::2, 0:64] = -gim.T
        gi[k1, 1::2, 64:128] = gr.T
    tb = lambda a: np.asarray(a, dtype=np.float32).astype(BF)
    return tb(rf), tb(ci), tb(fa), tb(gf), tb(gi)


_RF, _CI, _FA, _GF, _GI = _consts()


def _nn(a, b):
    return jnp.dot(a, b, preferred_element_type=F32)


def _nt(a, b):
    return lax.dot_general(a, b, (((1,), (1,)), ((), ())), preferred_element_type=F32)


BM = 512
XC = 512
NOB = 2


def _kernel(x_hbm, wr_hbm, wi_hbm, wg_hbm, wu_hbm, wd_hbm,
            rf_hbm, ci_hbm, fa_hbm, gf_hbm, gi_hbm,
            o_hbm,
            x_v, wr_v, wi_v, wg_v, wu_v, wd_v,
            rf_v, ci_v, fa_v, gf_v, gi_v,
            ze, zo, ye, yo, wsr, wsi,
            yre, yie, yro, yio, hh, ob,
            sem_x, sem_c, sem_o):

    def cp(src, dst, i):
        return pltpu.make_async_copy(src, dst, sem_c.at[i])

    nxc = S // XC
    xcp = [pltpu.make_async_copy(x_hbm.at[:, pl.ds(c * XC, XC)],
                                 x_v.at[:, pl.ds(c * XC, XC)], sem_x.at[c])
           for c in range(nxc)]
    c_rf = cp(rf_hbm, rf_v, 0)
    c_wr = cp(wr_hbm, wr_v, 1)
    c_wi = cp(wi_hbm, wi_v, 2)
    c_fa = cp(fa_hbm, fa_v, 3)
    c_gf = cp(gf_hbm, gf_v, 4)
    c_gi = cp(gi_hbm, gi_v, 5)
    c_ci = cp(ci_hbm, ci_v, 6)
    c_wg = cp(wg_hbm, wg_v, 7)
    c_wu = cp(wu_hbm, wu_v, 8)
    c_wd = cp(wd_hbm, wd_v, 9)

    xcp[0].start()
    c_rf.start()
    for c in range(1, nxc):
        xcp[c].start()
    c_fa.start()
    c_gf.start()

    c_rf.wait()
    for c in range(nxc):
        xcp[c].wait()
        if c == 0:
            c_wr.start()
            c_wi.start()
            c_gi.start()
            c_ci.start()
        if c == nxc - 1:
            c_wg.start()
            c_wu.start()
            c_wd.start()
        for tt in range(XC // 128):
            t = c * (XC // 128) + tt
            xt = x_v[:, t * 128:(t + 1) * 128].astype(F32)
            a0 = xt[:H] + xt[H:]
            b0 = xt[:H] - xt[H:]
            m2 = jnp.sum(a0, axis=0, keepdims=True) * (2.0 / D)
            ca = a0 - m2
            v = jnp.sum(ca * ca + b0 * b0, axis=0, keepdims=True) * (0.5 / D)
            r = lax.rsqrt(v + EPS)
            a = (ca * r).astype(BF)
            b = (b0 * r).astype(BF)
            ze_t = _nn(rf_v[0:256, 0:H], a)
            zo_t = _nn(rf_v[256:512, 0:H], b)
            we = pltpu.bitcast(ze_t.astype(BF), U32).T
            wo = pltpu.bitcast(zo_t.astype(BF), U32).T
            for g in range(2):
                ze[pl.ds(PZ * (2 * t + g), N2), :] = we[N2 * g:N2 * (g + 1)]
                zo[pl.ds(PZ * (2 * t + g), N2), :] = wo[N2 * g:N2 * (g + 1)]

    c_wr.wait()
    c_wi.wait()
    row8 = lax.broadcasted_iota(jnp.int32, (8, 128), 0)
    for src, dst in ((wr_v, wsr), (wi_v, wsi)):
        for t in range(S // 128):
            wd_ = pltpu.bitcast(src[0:H, t * 128:(t + 1) * 128], U32)
            ny = src[H:H + 1, t * 128:(t + 1) * 128].astype(F32)
            ny = pltpu.bitcast(jnp.broadcast_to(ny, (8, 128)), U32) >> 16
            ny = jnp.where(row8 == 0, ny, jnp.zeros_like(ny))
            wt = jnp.concatenate([wd_, ny, jnp.zeros((8, 128), U32)], axis=0).T
            for g in range(4):
                dst[pl.ds(PW * (4 * t + g), N1), :] = wt[N1 * g:N1 * (g + 1)]

    c_fa.wait()
    GA = 2
    for p0 in range(0, N2 // 2, GA):
        tiles = []
        for p in range(p0, p0 + GA):
            for z in (ze, zo):
                w = jnp.concatenate([z[pl.ds(2 * p, N1, stride=PZ), :],
                                     z[pl.ds(2 * p + 1, N1, stride=PZ), :]], axis=0)
                tiles.append(pltpu.bitcast(w, BF))
        res = _nn(fa_v[0], jnp.concatenate(tiles, axis=1))
        i = 0
        for p in range(p0, p0 + GA):
            for y in (ye, yo):
                w = pltpu.bitcast(res[:, i * 128:(i + 1) * 128].astype(BF), U32)
                y[pl.ds(2 * p, N1, stride=PZ), :] = w[:N1]
                y[pl.ds(2 * p + 1, N1, stride=PZ), :] = w[N1:]
                i += 1

    c_gf.wait()
    c_gi.wait()
    for k1 in range(N1):
        te = pltpu.bitcast(ye[pl.ds(PZ * k1, N2), :], BF)
        to = pltpu.bitcast(yo[pl.ds(PZ * k1, N2), :], BF)
        xx = _nn(gf_v[k1], jnp.concatenate([te, to], axis=1))
        wr = wsr[pl.ds(k1, N2, stride=PW), :]
        wi = wsi[pl.ds(k1, N2, stride=PW), :]
        wre = pltpu.bitcast(wr << 16, F32)
        wie = pltpu.bitcast(wi << 16, F32)
        wro = pltpu.bitcast(wr & jnp.uint32(0xFFFF0000), F32)
        wio = pltpu.bitcast(wi & jnp.uint32(0xFFFF0000), F32)
        xre, xie = xx[:N2, :128], xx[N2:, :128]
        xro, xio = xx[:N2, 128:], xx[N2:, 128:]
        pe = jnp.concatenate([xre * wre - xie * wie, xre * wie + xie * wre], axis=0)
        po = jnp.concatenate([xro * wro - xio * wio, xro * wio + xio * wro], axis=0)
        yy = _nn(gi_v[k1], jnp.concatenate([pe.astype(BF), po.astype(BF)], axis=1))
        ze[pl.ds(PZ * k1, N2), :] = pltpu.bitcast(yy[:, :128].astype(BF), U32)
        zo[pl.ds(PZ * k1, N2), :] = pltpu.bitcast(yy[:, 128:].astype(BF), U32)

    for p0 in range(0, N2 // 2, GA):
        tiles = []
        for p in range(p0, p0 + GA):
            for z in (ze, zo):
                w = jnp.concatenate([z[pl.ds(2 * p, N1, stride=PZ), :],
                                     z[pl.ds(2 * p + 1, N1, stride=PZ), :]], axis=0)
                tiles.append(pltpu.bitcast(w, BF))
        res = _nn(fa_v[1], jnp.concatenate(tiles, axis=1))
        i = 0
        for p in range(p0, p0 + GA):
            for (yr_, yi_) in ((yre, yie), (yro, yio)):
                w = pltpu.bitcast(res[:, i * 128:(i + 1) * 128].astype(BF), U32)
                yr_[pl.ds(p, N1, stride=PW), :] = w[:N1]
                yi_[pl.ds(p, N1, stride=PW), :] = w[N1:]
                i += 1

    c_ci.wait()
    c_wg.wait()
    c_wu.wait()
    c_wd.wait()
    nb = S // BM
    ocp = [pltpu.make_async_copy(ob.at[j % NOB], o_hbm.at[:, pl.ds(j * BM, BM)], sem_o.at[j % NOB])
           for j in range(nb)]
    for j in range(nb):
        def gather(yr_, yi_):
            rows = []
            for g in range(BM // N2):
                n1 = j * (BM // N2) + g
                rows.append(jnp.concatenate(
                    [pltpu.bitcast(yr_[pl.ds(PW * n1, N1), :], BF),
                     pltpu.bitcast(yi_[pl.ds(PW * n1, N1), :], BF)], axis=1))
            return jnp.concatenate(rows, axis=0)
        ep = _nt(ci_v[0], gather(yre, yie))
        op = _nt(ci_v[1], gather(yro, yio))
        xt = x_v[:, j * BM:(j + 1) * BM].astype(F32)
        h = jnp.concatenate([xt[:H] + (ep + op), xt[H:] + (ep - op)], axis=0)
        m = jnp.mean(h, axis=0, keepdims=True)
        cen = h - m
        v = jnp.mean(cen * cen, axis=0, keepdims=True)
        l2 = (cen * lax.rsqrt(v + EPS)).astype(BF).T
        g_ = _nn(l2, wg_v[...])
        u_ = _nn(l2, wu_v[...])
        hh[...] = (g_ * u_).astype(BF)
        o = _nt(wd_v[...], hh[...])
        if j >= NOB:
            ocp[j - NOB].wait()
        ob[j % NOB] = (h + o).astype(BF)
        ocp[j].start()
    for j in range(max(nb - NOB, 0), nb):
        ocp[j].wait()


@jax.jit
def pallas_sequential_preLN__spectral_gfnet__glu_gated_bilinear__prompt_kernel(
    A_x, A_w_r, A_w_i, B_x, B_w_gate, B_w_up, B_w_down,
):
    del B_x
    xT = jnp.transpose(A_x.reshape(S, D))
    any_spec = pl.BlockSpec(memory_space=pl.ANY)
    vm = pltpu.VMEM
    oT = pl.pallas_call(
        _kernel,
        out_shape=jax.ShapeDtypeStruct((D, S), BF),
        in_specs=[any_spec] * 11,
        out_specs=any_spec,
        scratch_shapes=[
            vm((D, S), BF), vm((H + 1, S), BF), vm((H + 1, S), BF),
            vm((D, FF), BF), vm((D, FF), BF), vm((D, FF), BF),
            vm(_RF.shape, BF), vm(_CI.shape, BF), vm(_FA.shape, BF),
            vm(_GF.shape, BF), vm(_GI.shape, BF),
            vm((N1 * PZ, 128), U32), vm((N1 * PZ, 128), U32),
            vm((N1 * PZ, 128), U32), vm((N1 * PZ, 128), U32),
            vm((N2 * PW, 128), U32), vm((N2 * PW, 128), U32),
            vm((N1 * PW, 128), U32), vm((N1 * PW, 128), U32),
            vm((N1 * PW, 128), U32), vm((N1 * PW, 128), U32),
            vm((BM, FF), BF), vm((NOB, D, BM), BF),
            pltpu.SemaphoreType.DMA((S // XC,)),
            pltpu.SemaphoreType.DMA((10,)),
            pltpu.SemaphoreType.DMA((NOB,)),
        ],
        compiler_params=pltpu.CompilerParams(vmem_limit_bytes=100 * 1024 * 1024),
        name="gfnet_glu",
    )(xT, A_w_r.T, A_w_i.T, B_w_gate, B_w_up, B_w_down.T, _RF, _CI, _FA, _GF, _GI)
    return jnp.transpose(oT).reshape(1, S, D)
```

```python
import numpy as np
import jax
import jax.numpy as jnp
from jax import lax
from jax.experimental import pallas as pl
from jax.experimental.pallas import tpu as pltpu

S, D, FF = 2048, 448, 1792
H = D // 2
N1, N2 = 32, 64
PZ = N2 + 1
PW = N1 + 1
BF = jnp.bfloat16
F32 = jnp.float32
U32 = jnp.uint32
EPS = 1e-5


def _consts():
    d = np.arange(H)
    rf = np.zeros((512, 256))
    for m in range(H // 2 + 1):
        ang = -2.0 * np.pi * ((2 * m * d) % D) / D
        rf[2 * m, :H] = np.cos(ang)
        rf[2 * m + 1, :H] = np.sin(ang)
    for m in range(H // 2):
        ang = -2.0 * np.pi * (((2 * m + 1) * d) % D) / D
        rf[256 + 2 * m, :H] = np.cos(ang)
        rf[256 + 2 * m + 1, :H] = np.sin(ang)
    ci = np.zeros((2, H, 256))
    for m in range(H // 2 + 1):
        k = 2 * m
        c = 1.0 if (k == 0 or k == H) else 2.0
        ang = 2.0 * np.pi * ((k * d) % D) / D
        ci[0, :, m] = c * np.cos(ang) / (S * D)
        if k != 0 and k != H:
            ci[0, :, 128 + m] = -c * np.sin(ang) / (S * D)
    for m in range(H // 2):
        k = 2 * m + 1
        ang = 2.0 * np.pi * ((k * d) % D) / D
        ci[1, :, m] = 2.0 * np.cos(ang) / (S * D)
        ci[1, :, 128 + m] = -2.0 * np.sin(ang) / (S * D)
    n1 = np.arange(N1)
    n2 = np.arange(N2)
    ang = -2.0 * np.pi * ((np.outer(n1, n1)) % N1) / N1
    fr, fi = np.cos(ang), np.sin(ang)
    fa = np.zeros((2, 128, 128))
    for mu in range(2):
        o = 64 * mu
        fa[0, o + 0:o + 64:2, o + 0:o + 64:2] = fr
        fa[0, o + 0:o + 64:2, o + 1:o + 64:2] = -fi
        fa[0, o + 1:o + 64:2, o + 0:o + 64:2] = fi
        fa[0, o + 1:o + 64:2, o + 1:o + 64:2] = fr
        fa[1, mu:64:2, o + 0:o + 64:2] = fr
        fa[1, mu:64:2, o + 1:o + 64:2] = fi
        fa[1, 64 + mu:128:2, o + 0:o + 64:2] = -fi
        fa[1, 64 + mu:128:2, o + 1:o + 64:2] = fr
    gf = np.zeros((N1, 128, 128))
    gi = np.zeros((N1, 128, 128))
    for k1 in range(N1):
        ang = -2.0 * np.pi * (np.outer(k1 + N1 * n2, n2) % S) / S
        gr, gim = np.cos(ang), np.sin(ang)
        gf[k1, 0:64, 0::2] = gr
        gf[k1, 0:64, 1::2] = -gim
        gf[k1, 64:128, 0::2] = gim
        gf[k1, 64:128, 1::2] = gr
        gi[k1, 0::2, 0:64] = gr.T
        gi[k1, 0::2, 64:128] = gim.T
        gi[k1, 1::2, 0:64] = -gim.T
        gi[k1, 1::2, 64:128] = gr.T
    tb = lambda a: np.asarray(a, dtype=np.float32).astype(BF)
    rf = np.stack([rf[:, :128], rf[:, 128:]])
    ci = np.stack([ci[0, :, :128], ci[0, :, 128:], ci[1, :, :128], ci[1, :, 128:]])
    return tb(rf), tb(ci), tb(fa), tb(gf)


_RF, _CI, _FA, _GF = _consts()


def _nn(a, b):
    return jnp.dot(a, b, preferred_element_type=F32)


def _nt(a, b):
    return lax.dot_general(a, b, (((1,), (1,)), ((), ())), preferred_element_type=F32)


def _tn(a, b):
    return lax.dot_general(a, b, (((0,), (0,)), ((), ())), preferred_element_type=F32)


def _run(g):
    for _ in g:
        pass


def _seq(*gs):
    for g in gs:
        yield from g


def _rr(*gs):
    gs = list(gs)
    while gs:
        nxt = []
        for g in gs:
            try:
                next(g)
                nxt.append(g)
            except StopIteration:
                pass
        gs = nxt
        yield


XC = 512
NXC = S // XC
NT = S // 128
TPC = XC // 128
BM = 256
NB = S // BM
NCH = FF // 256
CSPLIT = 4


def _take(g, n):
    for _ in range(n):
        try:
            next(g)
        except StopIteration:
            return
        yield


def _seven_b(b11, b12, b21, b22):
    return (b11 + b22, b11, b12 - b22, b21 - b11, b22, b11 + b12, b21 + b22)


def _seven_a(a11, a12, a21, a22):
    return (a11 + a22, a21 + a22, a11, a22, a11 + a12, a21 - a11, a12 - a22)


def _combine(m):
    return (m[0] + m[3] - m[4] + m[6], m[2] + m[4], m[1] + m[3], m[0] - m[1] + m[2] + m[5])


def _kernel(x_hbm, wr_hbm, wi_hbm, wg_hbm, wu_hbm, wd_hbm,
            rf_hbm, ci_hbm, fa_hbm, gf_hbm,
            o_hbm,
            x_v, wr_v, wi_v, wg_v, wu_v, wd_v,
            rf_v, ci_v, fa_v, gf_v,
            ab, ze, zo, ye, yo, wsr, wsi,
            yre, yie, yro, yio,
            hb, cn1, l2s, wgs, wus, wds, hs, ob,
            sem_x, sem_c, sem_o, sem_f):

    def colcp(src, dst, c0, w, sem):
        return pltpu.make_async_copy(src.at[:, pl.ds(c0, w)], dst.at[:, pl.ds(c0, w)], sem)

    xcp = [colcp(x_hbm, x_v, c * XC, XC, sem_x.at[c]) for c in range(NXC)]
    c_rf = pltpu.make_async_copy(rf_hbm, rf_v, sem_c.at[0])
    c_fa = pltpu.make_async_copy(fa_hbm, fa_v, sem_c.at[1])
    c_ci = pltpu.make_async_copy(ci_hbm, ci_v, sem_c.at[2])
    c_wr = pltpu.make_async_copy(wr_hbm, wr_v, sem_c.at[3])
    c_wi = pltpu.make_async_copy(wi_hbm, wi_v, sem_c.at[4])
    c_gf = pltpu.make_async_copy(gf_hbm, gf_v, sem_c.at[5])
    c_wd = pltpu.make_async_copy(wd_hbm, wd_v, sem_c.at[6])
    F0 = CSPLIT * 256
    wgc = [colcp(wg_hbm, wg_v, 0, F0, sem_c.at[7]), colcp(wg_hbm, wg_v, F0, FF - F0, sem_c.at[8])]
    wuc = [colcp(wu_hbm, wu_v, 0, F0, sem_c.at[9]), colcp(wu_hbm, wu_v, F0, FF - F0, sem_c.at[10])]
    ocp = [colcp(ob, o_hbm, j * BM, BM, sem_o.at[j]) for j in range(NB)]

    def ln1(t):
        xt = x_v[:, t * 128:(t + 1) * 128].astype(F32)
        a0 = xt[:H] + xt[H:]
        b0 = xt[:H] - xt[H:]
        yield
        m2 = jnp.sum(a0, axis=0, keepdims=True) * (2.0 / D)
        ca = a0 - m2
        yield
        v = jnp.sum(ca * ca + b0 * b0, axis=0, keepdims=True) * (0.5 / D)
        r = lax.rsqrt(v + EPS)
        yield
        ab[t, 0:H, :] = (ca * r).astype(BF)
        yield
        ab[t, H:D, :] = (b0 * r).astype(BF)

    def lhs2(ref, i, lo, hi):
        return jnp.concatenate([ref[i, lo:hi, :], ref[i + 1, lo:hi, :]], axis=1)

    def dfwd(t):
        for (lo, r0, dst) in ((0, 0, ze), (H, 256, zo)):
            res = _nn(lhs2(rf_v, 0, r0, r0 + 256)[:, :H], ab[t, lo:lo + H, :])
            yield
            w = pltpu.bitcast(res.astype(BF), U32).T
            for g in range(2):
                dst[pl.ds(PZ * (2 * t + g), N2), :] = w[N2 * g:N2 * (g + 1)]
            yield

    row8 = lax.broadcasted_iota(jnp.int32, (8, 128), 0)

    def wprep(t, src, dst):
        wd_ = pltpu.bitcast(src[0:H, t * 128:(t + 1) * 128], U32)
        ny = src[H:H + 1, t * 128:(t + 1) * 128].astype(F32)
        ny = pltpu.bitcast(jnp.broadcast_to(ny, (8, 128)), U32) >> 16
        ny = jnp.where(row8 == 0, ny, jnp.zeros_like(ny))
        wt = jnp.concatenate([wd_, ny, jnp.zeros((8, 128), U32)], axis=0).T
        for g in range(4):
            dst[pl.ds(PW * (4 * t + g), N1), :] = wt[N1 * g:N1 * (g + 1)]
        yield

    def gather32(ps):
        tiles = []
        for p in ps:
            for z in (ze, zo):
                w = jnp.concatenate([z[pl.ds(2 * p, N1, stride=PZ), :],
                                     z[pl.ds(2 * p + 1, N1, stride=PZ), :]], axis=0)
                tiles.append(pltpu.bitcast(w, BF))
        return jnp.concatenate(tiles, axis=1)

    def stage_a(ps):
        res = _nn(fa_v[0], gather32(ps))
        i = 0
        for p in ps:
            for y in (ye, yo):
                w = pltpu.bitcast(res[:, i * 128:(i + 1) * 128].astype(BF), U32)
                y[pl.ds(2 * p, N1, stride=PZ), :] = w[:N1]
                y[pl.ds(2 * p + 1, N1, stride=PZ), :] = w[N1:]
                i += 1
        yield

    def stage_b(k1):
        te = pltpu.bitcast(ye[pl.ds(PZ * k1, N2), :], BF)
        to = pltpu.bitcast(yo[pl.ds(PZ * k1, N2), :], BF)
        g = gf_v[k1]
        xx = _nn(g, jnp.concatenate([te, to], axis=1))
        wr = wsr[pl.ds(k1, N2, stride=PW), :]
        wi = wsi[pl.ds(k1, N2, stride=PW), :]
        wre = pltpu.bitcast(wr << 16, F32)
        wie = pltpu.bitcast(wi << 16, F32)
        wro = pltpu.bitcast(wr & jnp.uint32(0xFFFF0000), F32)
        wio = pltpu.bitcast(wi & jnp.uint32(0xFFFF0000), F32)
        xre, xie = xx[:N2, :128], xx[N2:, :128]
        xro, xio = xx[:N2, 128:], xx[N2:, 128:]
        pe = jnp.concatenate([xre * wre - xie * wie, xre * wie + xie * wre], axis=0)
        po = jnp.concatenate([xro * wro - xio * wio, xro * wio + xio * wro], axis=0)
        yy = _tn(g, jnp.concatenate([pe.astype(BF), po.astype(BF)], axis=1))
        ze[pl.ds(PZ * k1, N2), :] = pltpu.bitcast(yy[:, :128].astype(BF), U32)
        zo[pl.ds(PZ * k1, N2), :] = pltpu.bitcast(yy[:, 128:].astype(BF), U32)
        yield

    def stage_ai(ps):
        res = _nn(fa_v[1], gather32(ps))
        i = 0
        for p in ps:
            for (yr_, yi_) in ((yre, yie), (yro, yio)):
                w = pltpu.bitcast(res[:, i * 128:(i + 1) * 128].astype(BF), U32)
                yr_[pl.ds(p, N1, stride=PW), :] = w[:N1]
                yi_[pl.ds(p, N1, stride=PW), :] = w[N1:]
                i += 1
        yield

    def quads(src, c):
        f1, f2 = 256 * c, 256 * c + 128
        return (src[0:H, f1:f1 + 128].astype(F32), src[0:H, f2:f2 + 128].astype(F32),
                src[H:D, f1:f1 + 128].astype(F32), src[H:D, f2:f2 + 128].astype(F32))

    def wsprep(c):
        for src, dst in ((wg_v, wgs), (wu_v, wus)):
            ops = _seven_b(*quads(src, c))
            for i in range(7):
                dst[i, c] = ops[i].astype(BF)
            yield

    def wdprep(c):
        ops = _seven_a(*quads(wd_v, c))
        for i in range(7):
            wds[i, c] = ops[i].astype(BF)
        yield

    def prep(j):
        cn = []
        for i in range(2):
            t = 2 * j + i

            def gather(yr_, yi_):
                rows = []
                for g in range(2):
                    n1 = 2 * t + g
                    rows.append(jnp.concatenate(
                        [pltpu.bitcast(yr_[pl.ds(PW * n1, N1), :], BF),
                         pltpu.bitcast(yi_[pl.ds(PW * n1, N1), :], BF)], axis=1))
                return jnp.concatenate(rows, axis=0)
            ep = _nt(lhs2(ci_v, 0, 0, H), gather(yre, yie))
            op = _nt(lhs2(ci_v, 2, 0, H), gather(yro, yio))
            yield
            xt = x_v[:, t * 128:(t + 1) * 128].astype(F32)
            h = jnp.concatenate([xt[:H] + (ep + op), xt[H:] + (ep - op)], axis=0)
            hb[j % 2, i] = h.astype(BF)
            m = jnp.mean(h, axis=0, keepdims=True)
            cen = h - m
            yield
            v = jnp.mean(cen * cen, axis=0, keepdims=True)
            cn.append(cen * lax.rsqrt(v + EPS))
            if i == 0:
                cn1[...] = cn[0]
            yield
        c1 = cn1[...]
        c2 = cn[1]
        ops = _seven_a(c1[:H], c1[H:], c2[:H], c2[H:])
        for i in range(7):
            l2s[j % 2, i] = ops[i].astype(BF).T
            if i % 2 == 1:
                yield
        yield

    def gateup(j, c):
        quad = []
        for ws in (wgs, wus):
            quad.append(_combine([_nn(l2s[j % 2, i], ws[i, c]) for i in range(7)]))
            yield
        q11, q12, q21, q22 = [g_ * u_ for g_, u_ in zip(*quad)]
        ops = _seven_b(q11, q21, q12, q22)
        for i in range(7):
            hs[i, c] = ops[i].astype(BF)
        yield

    def down(j):
        m = []
        for i in range(7):
            lhs = jnp.concatenate([wds[i, c] for c in range(NCH)], axis=1)
            rhs = jnp.concatenate([hs[i, c] for c in range(NCH)], axis=1)
            m.append(_nt(lhs, rhs))
            if i % 2 == 1:
                yield
        o11, o12, o21, o22 = _combine(m)
        for i, (lo, hi) in enumerate(((o11, o21), (o12, o22))):
            t = 2 * j + i
            hh_ = hb[j % 2, i].astype(F32)
            ob[0:H, t * 128:(t + 1) * 128] = (hh_[:H] + lo).astype(BF)
            ob[H:D, t * 128:(t + 1) * 128] = (hh_[H:] + hi).astype(BF)
        ocp[j].start()
        yield

    for c in (xcp[0], c_rf, xcp[1], xcp[2], xcp[3], c_fa, c_wr, c_wi, c_gf, c_ci,
              wgc[0], wuc[0], wgc[1], wuc[1], c_wd):
        c.start()
        pl.semaphore_signal(sem_f, 1)
        pl.semaphore_wait(sem_f, 1)
    xcp[0].wait()
    _run(_seq(*[ln1(t) for t in range(TPC)]))
    c_rf.wait()
    for c in range(NXC):
        if c + 1 < NXC:
            xcp[c + 1].wait()
            _run(_rr(_seq(*[dfwd(t) for t in range(c * TPC, (c + 1) * TPC)]),
                     _seq(*[ln1(t) for t in range((c + 1) * TPC, (c + 2) * TPC)])))
        else:
            c_fa.wait()
            c_wr.wait()
            _run(_rr(_seq(*[dfwd(t) for t in range(c * TPC, (c + 1) * TPC)]),
                     _seq(*[wprep(t, wr_v, wsr) for t in range(NT // 2)])))
    GA = 2
    NG = (N2 // 2) // GA
    _run(_rr(_seq(*[stage_a([2 * g, 2 * g + 1]) for g in range(NG // 2)]),
             _seq(*[wprep(t, wr_v, wsr) for t in range(NT // 2, NT)])))
    c_wi.wait()
    _run(_rr(_seq(*[stage_a([2 * g, 2 * g + 1]) for g in range(NG // 2, NG)]),
             _seq(*[_seq(wprep(2 * t, wi_v, wsi), wprep(2 * t + 1, wi_v, wsi)) for t in range(NT // 2)])))
    c_gf.wait()
    for k1 in range(N1):
        _run(stage_b(k1))
    for g in range(NG):
        _run(stage_ai([2 * g, 2 * g + 1]))
    c_ci.wait()
    wgc[0].wait()
    wuc[0].wait()
    _run(_rr(prep(0), _seq(wsprep(0), wsprep(1))))
    for j in range(NB):
        nxt = prep(j + 1) if j + 1 < NB else _seq()
        if j == 0:
            _run(_rr(_seq(gateup(0, 0), gateup(0, 1)), _seq(wsprep(2), wsprep(3)), _take(nxt, 3)))
            wgc[1].wait()
            wuc[1].wait()
            c_wd.wait()
            _run(_rr(_seq(*[gateup(0, c) for c in range(2, NCH)], down(0)),
                     _seq(*[wsprep(c) for c in range(CSPLIT, NCH)], *[wdprep(c) for c in range(NCH)]),
                     nxt))
        else:
            _run(_rr(_seq(*[gateup(j, c) for c in range(NCH)], down(j)), nxt))
    for j in range(NB):
        ocp[j].wait()


@jax.jit
def pallas_sequential_preLN__spectral_gfnet__glu_gated_bilinear__prompt_kernel(
    A_x, A_w_r, A_w_i, B_x, B_w_gate, B_w_up, B_w_down,
):
    del B_x
    xT = jnp.transpose(A_x.reshape(S, D))
    any_spec = pl.BlockSpec(memory_space=pl.ANY)
    vm = pltpu.VMEM
    dma = pltpu.SemaphoreType.DMA
    oT = pl.pallas_call(
        _kernel,
        out_shape=jax.ShapeDtypeStruct((D, S), BF),
        in_specs=[any_spec] * 10,
        out_specs=any_spec,
        scratch_shapes=[
            vm((D, S), BF), vm((H + 1, S), BF), vm((H + 1, S), BF),
            vm((D, FF), BF), vm((D, FF), BF), vm((D, FF), BF),
            vm(_RF.shape, BF), vm(_CI.shape, BF), vm(_FA.shape, BF), vm(_GF.shape, BF),
            vm((NT, D, 128), BF),
            vm((N1 * PZ, 128), U32), vm((N1 * PZ, 128), U32),
            vm((N1 * PZ, 128), U32), vm((N1 * PZ, 128), U32),
            vm((N2 * PW, 128), U32), vm((N2 * PW, 128), U32),
            vm((N1 * PW, 128), U32), vm((N1 * PW, 128), U32),
            vm((N1 * PW, 128), U32), vm((N1 * PW, 128), U32),
            vm((2, 2, D, 128), BF), vm((D, 128), F32), vm((2, 7, 128, H), BF),
            vm((7, NCH, H, 128), BF), vm((7, NCH, H, 128), BF), vm((7, NCH, H, 128), BF),
            vm((7, NCH, 128, 128), BF), vm((D, S), BF),
            dma((NXC,)), dma((11,)), dma((NB,)), pltpu.SemaphoreType.REGULAR,
        ],
        compiler_params=pltpu.CompilerParams(vmem_limit_bytes=100 * 1024 * 1024),
        name="gfnet_glu",
    )(xT, A_w_r.T, A_w_i.T, B_w_gate, B_w_up, B_w_down.T, _RF, _CI, _FA, _GF)
    return jnp.transpose(oT).reshape(1, S, D)
```

```python
import numpy as np
import jax
import jax.numpy as jnp
from jax import lax
from jax.experimental import pallas as pl
from jax.experimental.pallas import tpu as pltpu

S, D, FF = 2048, 448, 1792
H = D // 2
N1, N2 = 32, 64
PZ = N2 + 1
PW = N1 + 1
PY = N2 + 4
BF = jnp.bfloat16
F32 = jnp.float32
U32 = jnp.uint32
EPS = 1e-5


def _consts():
    d = np.arange(H)
    rf = np.zeros((512, 256))
    for m in range(H // 2 + 1):
        ang = -2.0 * np.pi * ((2 * m * d) % D) / D
        rf[2 * m, :H] = np.cos(ang)
        rf[2 * m + 1, :H] = np.sin(ang)
    for m in range(H // 2):
        ang = -2.0 * np.pi * (((2 * m + 1) * d) % D) / D
        rf[256 + 2 * m, :H] = np.cos(ang)
        rf[256 + 2 * m + 1, :H] = np.sin(ang)
    ci = np.zeros((2, H, 256))
    for m in range(H // 2 + 1):
        k = 2 * m
        c = 1.0 if (k == 0 or k == H) else 2.0
        ang = 2.0 * np.pi * ((k * d) % D) / D
        ci[0, :, m] = c * np.cos(ang) / (S * D)
        if k != 0 and k != H:
            ci[0, :, 128 + m] = -c * np.sin(ang) / (S * D)
    for m in range(H // 2):
        k = 2 * m + 1
        ang = 2.0 * np.pi * ((k * d) % D) / D
        ci[1, :, m] = 2.0 * np.cos(ang) / (S * D)
        ci[1, :, 128 + m] = -2.0 * np.sin(ang) / (S * D)
    n1 = np.arange(N1)
    n2 = np.arange(N2)
    ang = -2.0 * np.pi * ((np.outer(n1, n1)) % N1) / N1
    fr, fi = np.cos(ang), np.sin(ang)
    fa = np.zeros((2, 128, 128))
    for mu in range(2):
        o = 64 * mu
        fa[0, o + 0:o + 64:2, o + 0:o + 64:2] = fr
        fa[0, o + 0:o + 64:2, o + 1:o + 64:2] = -fi
        fa[0, o + 1:o + 64:2, o + 0:o + 64:2] = fi
        fa[0, o + 1:o + 64:2, o + 1:o + 64:2] = fr
        fa[1, mu:64:2, o + 0:o + 64:2] = fr
        fa[1, mu:64:2, o + 1:o + 64:2] = fi
        fa[1, 64 + mu:128:2, o + 0:o + 64:2] = -fi
        fa[1, 64 + mu:128:2, o + 1:o + 64:2] = fr
    ang = -2.0 * np.pi * (np.outer(n2, n2) % N2) / N2
    fr, fi = np.cos(ang), np.sin(ang)
    pq = np.zeros((2, 128, 128))
    pq[0, 0:64, 0::2], pq[1, 0:64, 0::2] = fr, -fi
    pq[0, 0:64, 1::2], pq[1, 0:64, 1::2] = -fi, -fr
    pq[0, 64:128, 0::2], pq[1, 64:128, 0::2] = fi, fr
    pq[0, 64:128, 1::2], pq[1, 64:128, 1::2] = fr, -fi
    ang = -2.0 * np.pi * np.outer(n1, n2) / S
    tw = np.stack([np.repeat(np.cos(ang), 2, axis=1), np.repeat(np.sin(ang), 2, axis=1)])
    gt = np.concatenate([pq.reshape(256, 128), tw.reshape(64, 128)]).astype(np.float32)
    tb = lambda a: np.asarray(a, dtype=np.float32).astype(BF)
    rf = np.stack([rf[:, :128], rf[:, 128:]])
    ci = np.stack([ci[0, :, :128], ci[0, :, 128:], ci[1, :, :128], ci[1, :, 128:]])
    return tb(rf), tb(ci), tb(fa), gt


_RF, _CI, _FA, _GT = _consts()


def _nn(a, b):
    return jnp.dot(a, b, preferred_element_type=F32)


def _nt(a, b):
    return lax.dot_general(a, b, (((1,), (1,)), ((), ())), preferred_element_type=F32)


def _tn(a, b):
    return lax.dot_general(a, b, (((0,), (0,)), ((), ())), preferred_element_type=F32)


def _run(g):
    for _ in g:
        pass


def _seq(*gs):
    for g in gs:
        yield from g


def _rr(*gs):
    gs = list(gs)
    while gs:
        nxt = []
        for g in gs:
            try:
                next(g)
                nxt.append(g)
            except StopIteration:
                pass
        gs = nxt
        yield


XC = 512
NXC = S // XC
NT = S // 128
TPC = XC // 128
BM = 256
NB = S // BM
NCH = FF // 256
CSPLIT = 4


def _take(g, n):
    for _ in range(n):
        try:
            next(g)
        except StopIteration:
            return
        yield


def _mix(ga, na, gb, nb):
    k = 0
    for a in range(na):
        next(ga, None)
        while k < (a + 1) * nb // na:
            next(gb, None)
            k += 1
        yield
    _run(ga)
    _run(gb)


def _seven_b(b11, b12, b21, b22):
    return (b11 + b22, b11, b12 - b22, b21 - b11, b22, b11 + b12, b21 + b22)


def _seven_a(a11, a12, a21, a22):
    return (a11 + a22, a21 + a22, a11, a22, a11 + a12, a21 - a11, a12 - a22)


TERMS_A = ((0, (1, 3)), (2, (1, 3)), (0,), (3,), (0, (1, 1)), (2, (-1, 0)), (1, (-1, 3)))
TERMS_B = ((0, (1, 3)), (0,), (1, (-1, 3)), (2, (-1, 0)), (3,), (0, (1, 1)), (2, (1, 3)))


def _combine(m):
    return (m[0] + m[3] - m[4] + m[6], m[2] + m[4], m[1] + m[3], m[0] - m[1] + m[2] + m[5])


def _words(ref):
    return ref.bitcast(U32)


def _bf(w):
    return pltpu.bitcast(w, BF)


def _kernel(x_hbm, wr_hbm, wi_hbm, wg_hbm, wu_hbm, wd_hbm,
            rf_hbm, ci_hbm, fa_hbm, gt_hbm,
            o_hbm,
            x_v, wr_v, wi_v, wg_v, wu_v, wd_v,
            rf_v, ci_v, fa_v, gt_v,
            ab, zt, ze, zo, ye, yo, ve, vo, wsr, wsi, se, so,
            hb, cn1, l2a, l2b, wgs, wus, wds, hs, ob,
            sem_x, sem_c, sem_o, sem_f):

    def colcp(src, dst, c0, w, sem):
        return pltpu.make_async_copy(src.at[:, pl.ds(c0, w)], dst.at[:, pl.ds(c0, w)], sem)

    xcp = [colcp(x_hbm, x_v, c * XC, XC, sem_x.at[c]) for c in range(NXC)]
    c_rf = pltpu.make_async_copy(rf_hbm, rf_v, sem_c.at[0])
    c_fa = pltpu.make_async_copy(fa_hbm, fa_v, sem_c.at[1])
    c_ci = pltpu.make_async_copy(ci_hbm, ci_v, sem_c.at[2])
    c_wr = pltpu.make_async_copy(wr_hbm, wr_v, sem_c.at[3])
    c_wi = pltpu.make_async_copy(wi_hbm, wi_v, sem_c.at[4])
    c_gt = pltpu.make_async_copy(gt_hbm, gt_v, sem_c.at[5])
    c_wd = pltpu.make_async_copy(wd_hbm, wd_v, sem_c.at[6])
    F0 = CSPLIT * 256
    wgc = [colcp(wg_hbm, wg_v, 0, F0, sem_c.at[7]), colcp(wg_hbm, wg_v, F0, FF - F0, sem_c.at[8])]
    wuc = [colcp(wu_hbm, wu_v, 0, F0, sem_c.at[9]), colcp(wu_hbm, wu_v, F0, FF - F0, sem_c.at[10])]
    ocp = [colcp(ob, o_hbm, j * BM, BM, sem_o.at[j]) for j in range(NB)]

    rf_w, ci_w, fa_w = _words(rf_v), _words(ci_v), _words(fa_v)
    ab_w, zt_w = _words(ab), _words(zt)
    ye_w, yo_w, ve_w, vo_w, se_w, so_w = (_words(r) for r in (ye, yo, ve, vo, se, so))
    hb_w, l2a_w, l2b_w = _words(hb), _words(l2a), _words(l2b)
    wgs_w, wus_w, wds_w, hs_w = _words(wgs), _words(wus), _words(wds), _words(hs)

    def ln1(t):
        xt = x_v[:, t * 128:(t + 1) * 128].astype(F32)
        a0 = xt[:H] + xt[H:]
        b0 = xt[:H] - xt[H:]
        yield
        m2 = jnp.sum(a0, axis=0, keepdims=True) * (2.0 / D)
        ca = a0 - m2
        yield
        v = jnp.sum(ca * ca + b0 * b0, axis=0, keepdims=True) * (0.5 / D)
        r = lax.rsqrt(v + EPS)
        yield
        ab[t, 0:H, :] = (ca * r).astype(BF)
        yield
        ab[t, H:D, :] = (b0 * r).astype(BF)

    def dfwd(t):
        for (e, dst) in ((0, ze), (1, zo)):
            lhs = jnp.concatenate([_bf(rf_w[0, e * 128:(e + 1) * 128, :]),
                                   _bf(rf_w[1, e * 128:(e + 1) * 128, :])[:, :H - 128]], axis=1)
            res = _nn(lhs, _bf(ab_w[t, e * (H // 2):(e + 1) * (H // 2), :]))
            zt[t, e] = res.astype(BF)
            yield
            w = zt_w[t, e].T
            for g in range(2):
                dst[pl.ds(PZ * (2 * t + g), N2), :] = w[N2 * g:N2 * (g + 1)]
            yield

    row8 = lax.broadcasted_iota(jnp.int32, (8, 128), 0)

    def wprep(t, src, dst):
        wd_ = pltpu.bitcast(src[0:H, t * 128:(t + 1) * 128], U32)
        ny = src[H:H + 1, t * 128:(t + 1) * 128].astype(F32)
        ny = pltpu.bitcast(jnp.broadcast_to(ny, (8, 128)), U32) >> 16
        ny = jnp.where(row8 == 0, ny, jnp.zeros_like(ny))
        wt = jnp.concatenate([wd_, ny, jnp.zeros((8, 128), U32)], axis=0).T
        for g in range(4):
            dst[pl.ds(PW * (4 * t + g), N1), :] = wt[N1 * g:N1 * (g + 1)]
        yield

    def gather2(src, s0, s1, pitch):
        return _bf(jnp.concatenate([src[pl.ds(s0, N1, stride=pitch), :],
                                    src[pl.ds(s1, N1, stride=pitch), :]], axis=0))

    def stage_a(ps):
        rhs = jnp.concatenate([gather2(z, p, p + N1, PZ) for p in ps for z in (ze, zo)], axis=1)
        res = _nn(_bf(fa_w[0]), rhs)
        i = 0
        for p in ps:
            for y in (ye, yo):
                y[pl.ds(2 * PY * p, 128), :] = res[:, i * 128:(i + 1) * 128].astype(BF)
                i += 1
        yield

    def stage_b(k1):
        g = (gt_v[0:128, :] * gt_v[256 + k1:257 + k1, :]
             + gt_v[128:256, :] * gt_v[288 + k1:289 + k1, :]).astype(BF)
        rhs = jnp.concatenate([gather2(y, k1, N1 + k1, PY) for y in (ye_w, yo_w)], axis=1)
        xx = _nn(g, rhs)
        wr = wsr[pl.ds(k1, N2, stride=PW), :]
        wi = wsi[pl.ds(k1, N2, stride=PW), :]
        wre = pltpu.bitcast(wr << 16, F32)
        wie = pltpu.bitcast(wi << 16, F32)
        wro = pltpu.bitcast(wr & jnp.uint32(0xFFFF0000), F32)
        wio = pltpu.bitcast(wi & jnp.uint32(0xFFFF0000), F32)
        xre, xie = xx[:N2, :128], xx[N2:, :128]
        xro, xio = xx[:N2, 128:], xx[N2:, 128:]
        pe = jnp.concatenate([xre * wre - xie * wie, xre * wie + xie * wre], axis=0)
        po = jnp.concatenate([xro * wro - xio * wio, xro * wio + xio * wro], axis=0)
        yy = _nn(g.T, jnp.concatenate([pe.astype(BF), po.astype(BF)], axis=1))
        ve[pl.ds(2 * PY * k1, 128), :] = yy[:, :128].astype(BF)
        vo[pl.ds(2 * PY * k1, 128), :] = yy[:, 128:].astype(BF)
        yield

    def stage_ai(ps):
        rhs = jnp.concatenate([gather2(v, 2 * p, 2 * p + 1, PY) for p in ps for v in (ve_w, vo_w)],
                              axis=1)
        res = _nn(_bf(fa_w[1]), rhs)
        i = 0
        for p in ps:
            for y in (se, so):
                y[pl.ds(2 * PY * p, 128), :] = res[:, i * 128:(i + 1) * 128].astype(BF)
                i += 1
        yield

    def quad(src, c, q):
        r0, f0 = (q // 2) * H, 256 * c + (q % 2) * 128
        return src[r0:r0 + H, f0:f0 + 128].astype(F32)

    def operand(j, src, dst, dst_w, terms, i, c):
        if j > 0:
            return _bf(dst_w[i, c])
        v = quad(src, c, terms[i][0])
        for sign, q in terms[i][1:]:
            v = v + quad(src, c, q) if sign > 0 else v - quad(src, c, q)
        v = v.astype(BF)
        dst[i, c] = v
        return v

    def prep(j):
        cn = []
        for i in range(2):
            t = 2 * j + i

            def inv_d(e, src):
                rhs = jnp.concatenate(
                    [_bf(jnp.concatenate([src[pl.ds(ro * N1 + 2 * t + g, N1, stride=PY), :]
                                          for g in range(2)], axis=0))
                     for ro in range(2)], axis=1)
                lhs = jnp.concatenate([_bf(ci_w[2 * e]), _bf(ci_w[2 * e + 1])], axis=1)
                return _nt(lhs, rhs)
            ep = inv_d(0, se_w)
            op = inv_d(1, so_w)
            yield
            xt = x_v[:, t * 128:(t + 1) * 128].astype(F32)
            h = jnp.concatenate([xt[:H] + (ep + op), xt[H:] + (ep - op)], axis=0)
            hb[j % 2, i] = h.astype(BF)
            m = jnp.mean(h, axis=0, keepdims=True)
            cen = h - m
            yield
            v = jnp.mean(cen * cen, axis=0, keepdims=True)
            cn.append(cen * lax.rsqrt(v + EPS))
            if i == 0:
                cn1[...] = cn[0]
            yield
        c1 = cn1[...]
        c2 = cn[1]
        ops = _seven_a(c1[:H], c1[H:], c2[:H], c2[H:])
        zpad = jnp.zeros((256 - H, 128), F32)
        for i in range(7):
            l2a_w[j % 2, i] = pltpu.bitcast(ops[i][:128].astype(BF).T, U32)
            l2b_w[j % 2, i] = pltpu.bitcast(
                jnp.concatenate([ops[i][128:], zpad], axis=0).astype(BF).T, U32)
            if i % 2 == 1:
                yield
        yield

    def gateup(j, c):
        quad = []
        for w_v, ws, ws_w in ((wg_v, wgs, wgs_w), (wu_v, wus, wus_w)):
            m = []
            for i in range(7):
                lhs = jnp.concatenate([_bf(l2a_w[j % 2, i]), _bf(l2b_w[j % 2, i])[:, :H - 128]], axis=1)
                m.append(_nn(lhs, operand(j, w_v, ws, ws_w, TERMS_B, i, c)))
            quad.append(_combine(m))
            yield
        q11, q12, q21, q22 = [g_ * u_ for g_, u_ in zip(*quad)]
        ops = _seven_b(q11, q21, q12, q22)
        for i in range(7):
            hs[i, c] = ops[i].astype(BF)
        yield

    def down(j):
        m = []
        for i in range(7):
            lhs = jnp.concatenate([operand(j, wd_v, wds, wds_w, TERMS_A, i, c) for c in range(NCH)],
                                  axis=1)
            rhs = jnp.concatenate([_bf(hs_w[i, c]) for c in range(NCH)], axis=1)
            m.append(_nt(lhs, rhs))
            if i % 2 == 1:
                yield
        o11, o12, o21, o22 = _combine(m)
        for i, (lo, hi) in enumerate(((o11, o21), (o12, o22))):
            t = 2 * j + i
            hh_ = _bf(hb_w[j % 2, i]).astype(F32)
            ob[0:H, t * 128:(t + 1) * 128] = (hh_[:H] + lo).astype(BF)
            ob[H:D, t * 128:(t + 1) * 128] = (hh_[H:] + hi).astype(BF)
        ocp[j].start()
        yield

    for c in (xcp[0], c_rf, xcp[1], xcp[2], xcp[3], c_fa, c_wr, c_wi, c_gt, c_ci,
              wgc[0], wuc[0], wgc[1], wuc[1], c_wd):
        c.start()
        pl.semaphore_signal(sem_f, 1)
        pl.semaphore_wait(sem_f, 1)
    for c in range(NXC):
        xcp[c].wait()
        if c == 0:
            seed = x_v[0:8, 0:128]
            for buf in (ab, zt, hb, l2a, l2b, wgs, wus, wds, hs):
                buf[(0,) * (len(buf.shape) - 2) + (slice(0, 8), slice(None))] = seed
            c_rf.wait()
        for t in range(c * TPC, (c + 1) * TPC):
            _run(ln1(t))
            _run(dfwd(t))
    NG = N1 // 2
    c_fa.wait()
    c_wr.wait()
    _run(_mix(_seq(*[stage_a([2 * g, 2 * g + 1]) for g in range(NG // 2)]), NG // 2,
              _seq(*[wprep(t, wr_v, wsr) for t in range(NT)]), NT))
    c_wi.wait()
    _run(_mix(_seq(*[stage_a([2 * g, 2 * g + 1]) for g in range(NG // 2, NG)]), NG // 2,
              _seq(*[wprep(t, wi_v, wsi) for t in range(NT)]), NT))
    c_gt.wait()
    for k1 in range(N1):
        _run(stage_b(k1))
    for g in range(NG):
        _run(stage_ai([2 * g, 2 * g + 1]))
    c_ci.wait()
    wgc[0].wait()
    wuc[0].wait()
    _run(prep(0))
    for j in range(NB):
        nxt = prep(j + 1) if j + 1 < NB else _seq()
        if j == 0:
            _run(_rr(_seq(*[gateup(0, c) for c in range(CSPLIT)]), _take(nxt, 6)))
            wgc[1].wait()
            wuc[1].wait()
            _run(_rr(_seq(*[gateup(0, c) for c in range(CSPLIT, NCH)]), nxt))
            c_wd.wait()
            _run(down(0))
        else:
            _run(_rr(_seq(*[gateup(j, c) for c in range(NCH)], down(j)), nxt))
    for j in range(NB):
        ocp[j].wait()


def _skip(n):
    for _ in range(n):
        yield


@jax.jit
def pallas_sequential_preLN__spectral_gfnet__glu_gated_bilinear__prompt_kernel(
    A_x, A_w_r, A_w_i, B_x, B_w_gate, B_w_up, B_w_down,
):
    del B_x
    xT = jnp.transpose(A_x.reshape(S, D))
    any_spec = pl.BlockSpec(memory_space=pl.ANY)
    vm = pltpu.VMEM
    dma = pltpu.SemaphoreType.DMA
    slab = vm((2 * PY * N1, 128), BF)
    oT = pl.pallas_call(
        _kernel,
        out_shape=jax.ShapeDtypeStruct((D, S), BF),
        in_specs=[any_spec] * 10,
        out_specs=any_spec,
        scratch_shapes=[
            vm((D, S), BF), vm((H + 1, S), BF), vm((H + 1, S), BF),
            vm((D, FF), BF), vm((D, FF), BF), vm((D, FF), BF),
            vm(_RF.shape, BF), vm(_CI.shape, BF), vm(_FA.shape, BF), vm(_GT.shape, F32),
            vm((NT, D, 128), BF), vm((NT, 2, 256, 128), BF),
            vm((N1 * PZ, 128), U32), vm((N1 * PZ, 128), U32),
            slab, slab, slab, slab,
            vm((N2 * PW, 128), U32), vm((N2 * PW, 128), U32),
            slab, slab,
            vm((2, 2, D, 128), BF), vm((D, 128), F32),
            vm((2, 7, 128, 128), BF), vm((2, 7, 128, 128), BF),
            vm((7, NCH, H, 128), BF), vm((7, NCH, H, 128), BF), vm((7, NCH, H, 128), BF),
            vm((7, NCH, 128, 128), BF), vm((D, S), BF),
            dma((NXC,)), dma((11,)), dma((NB,)), pltpu.SemaphoreType.REGULAR,
        ],
        compiler_params=pltpu.CompilerParams(vmem_limit_bytes=100 * 1024 * 1024),
        name="gfnet_glu",
    )(xT, A_w_r.T, A_w_i.T, B_w_gate, B_w_up, B_w_down.T, _RF, _CI, _FA, _GT)
    return jnp.transpose(oT).reshape(1, S, D)
```

```python
import numpy as np
import jax
import jax.numpy as jnp
from jax import lax
from jax.experimental import pallas as pl
from jax.experimental.pallas import tpu as pltpu

S, D, FF = 2048, 448, 1792
H = D // 2
N1, N2 = 32, 64
PZ = N2 + 1
PW = N1 + 1
PY = N2 + 4
BF = jnp.bfloat16
F32 = jnp.float32
U32 = jnp.uint32
EPS = 1e-5


def _consts():
    d = np.arange(H)
    rf = np.zeros((512, 256))
    for m in range(H // 2 + 1):
        ang = -2.0 * np.pi * ((2 * m * d) % D) / D
        rf[2 * m, :H] = np.cos(ang)
        rf[2 * m + 1, :H] = np.sin(ang)
    for m in range(H // 2):
        ang = -2.0 * np.pi * (((2 * m + 1) * d) % D) / D
        rf[256 + 2 * m, :H] = np.cos(ang)
        rf[256 + 2 * m + 1, :H] = np.sin(ang)
    ci = np.zeros((2, H, 256))
    for m in range(H // 2 + 1):
        k = 2 * m
        c = 1.0 if (k == 0 or k == H) else 2.0
        ang = 2.0 * np.pi * ((k * d) % D) / D
        ci[0, :, m] = c * np.cos(ang) / (S * D)
        if k != 0 and k != H:
            ci[0, :, 128 + m] = -c * np.sin(ang) / (S * D)
    for m in range(H // 2):
        k = 2 * m + 1
        ang = 2.0 * np.pi * ((k * d) % D) / D
        ci[1, :, m] = 2.0 * np.cos(ang) / (S * D)
        ci[1, :, 128 + m] = -2.0 * np.sin(ang) / (S * D)
    n1 = np.arange(N1)
    n2 = np.arange(N2)
    ang = -2.0 * np.pi * ((np.outer(n1, n1)) % N1) / N1
    fr, fi = np.cos(ang), np.sin(ang)
    fa = np.zeros((2, 128, 128))
    for mu in range(2):
        o = 64 * mu
        fa[0, o + 0:o + 64:2, o + 0:o + 64:2] = fr
        fa[0, o + 0:o + 64:2, o + 1:o + 64:2] = -fi
        fa[0, o + 1:o + 64:2, o + 0:o + 64:2] = fi
        fa[0, o + 1:o + 64:2, o + 1:o + 64:2] = fr
        fa[1, mu:64:2, o + 0:o + 64:2] = fr
        fa[1, mu:64:2, o + 1:o + 64:2] = fi
        fa[1, 64 + mu:128:2, o + 0:o + 64:2] = -fi
        fa[1, 64 + mu:128:2, o + 1:o + 64:2] = fr
    ang = -2.0 * np.pi * (np.outer(n2, n2) % N2) / N2
    fr, fi = np.cos(ang), np.sin(ang)
    pq = np.zeros((2, 128, 128))
    pq[0, 0:64, 0::2], pq[1, 0:64, 0::2] = fr, -fi
    pq[0, 0:64, 1::2], pq[1, 0:64, 1::2] = -fi, -fr
    pq[0, 64:128, 0::2], pq[1, 64:128, 0::2] = fi, fr
    pq[0, 64:128, 1::2], pq[1, 64:128, 1::2] = fr, -fi
    ang = -2.0 * np.pi * np.outer(n1, n2) / S
    tw = np.stack([np.repeat(np.cos(ang), 2, axis=1), np.repeat(np.sin(ang), 2, axis=1)])
    gt = np.concatenate([pq.reshape(256, 128), tw.reshape(64, 128)]).astype(np.float32)
    tb = lambda a: np.asarray(a, dtype=np.float32).astype(BF)
    rf = np.stack([rf[:, :128], rf[:, 128:]])
    ci = np.stack([ci[0, :, :128], ci[0, :, 128:], ci[1, :, :128], ci[1, :, 128:]])
    return tb(rf), tb(ci), tb(fa), gt


_RF, _CI, _FA, _GT = _consts()


def _nn(a, b):
    return jnp.dot(a, b, preferred_element_type=F32)


def _nt(a, b):
    return lax.dot_general(a, b, (((1,), (1,)), ((), ())), preferred_element_type=F32)


def _tn(a, b):
    return lax.dot_general(a, b, (((0,), (0,)), ((), ())), preferred_element_type=F32)


def _run(g):
    for _ in g:
        pass


def _seq(*gs):
    for g in gs:
        yield from g


def _rr(*gs):
    gs = list(gs)
    while gs:
        nxt = []
        for g in gs:
            try:
                next(g)
                nxt.append(g)
            except StopIteration:
                pass
        gs = nxt
        yield


NT = S // 128
XT = (0, 4, 8, 16)
NXC = len(XT) - 1
BM = 512
NB = S // BM
Q = D // 4
NC2 = 3
F1 = 512 * NC2
F0 = 1024
NKT = FF // 256


def _take(g, n):
    for _ in range(n):
        try:
            next(g)
        except StopIteration:
            return
        yield


def _mix(ga, na, gb, nb):
    k = 0
    for a in range(na):
        next(ga, None)
        while k < (a + 1) * nb // na:
            next(gb, None)
            k += 1
        yield
    _run(ga)
    _run(gb)


def _seven_b(b11, b12, b21, b22):
    return (b11 + b22, b11, b12 - b22, b21 - b11, b22, b11 + b12, b21 + b22)


def _seven_a(a11, a12, a21, a22):
    return (a11 + a22, a21 + a22, a11, a22, a11 + a12, a21 - a11, a12 - a22)


TERMS_A = (((1, 0), (1, 3)), ((1, 2), (1, 3)), ((1, 0),), ((1, 3),),
           ((1, 0), (1, 1)), ((1, 2), (-1, 0)), ((1, 1), (-1, 3)))
TERMS_B = (((1, 0), (1, 3)), ((1, 0),), ((1, 1), (-1, 3)), ((1, 2), (-1, 0)),
           ((1, 3),), ((1, 0), (1, 1)), ((1, 2), (1, 3)))


def _term(terms, get):
    v = get(terms[0][1])
    for sign, q in terms[1:]:
        v = v + get(q) if sign > 0 else v - get(q)
    return v


def _combine(m):
    return (m[0] + m[3] - m[4] + m[6], m[2] + m[4], m[1] + m[3], m[0] - m[1] + m[2] + m[5])


def _words(ref):
    return ref.bitcast(U32)


def _bf(w):
    return pltpu.bitcast(w, BF)


def _kernel(x_hbm, wr_hbm, wi_hbm, wg_hbm, wu_hbm, wd_hbm,
            rf_hbm, ci_hbm, fa_hbm, gt_hbm,
            o_hbm,
            x_v, wr_v, wi_v, wg_v, wu_v, wd_v,
            rf_v, ci_v, fa_v, gt_v, gs, xs,
            ab, zt, ze, zo, ye, yo, ve, vo, wsr, wsi, se, so,
            hb, cn, a2, a1, wg2, wu2, wg1, wu1, wds, hs, ob,
            sem_x, sem_c, sem_o, sem_f):

    def colcp(src, dst, c0, w, sem):
        return pltpu.make_async_copy(src.at[:, pl.ds(c0, w)], dst.at[:, pl.ds(c0, w)], sem)

    xcp = [colcp(x_hbm, x_v, XT[c] * 128, (XT[c + 1] - XT[c]) * 128, sem_x.at[c])
           for c in range(NXC)]
    c_rf = pltpu.make_async_copy(rf_hbm, rf_v, sem_c.at[0])
    c_fa = pltpu.make_async_copy(fa_hbm, fa_v, sem_c.at[1])
    c_ci = pltpu.make_async_copy(ci_hbm, ci_v, sem_c.at[2])
    c_wr = pltpu.make_async_copy(wr_hbm, wr_v, sem_c.at[3])
    c_wi = pltpu.make_async_copy(wi_hbm, wi_v, sem_c.at[4])
    c_gt = pltpu.make_async_copy(gt_hbm, gt_v, sem_c.at[5])
    c_wd = pltpu.make_async_copy(wd_hbm, wd_v, sem_c.at[6])
    wgc = [colcp(wg_hbm, wg_v, 0, F0, sem_c.at[7]), colcp(wg_hbm, wg_v, F0, FF - F0, sem_c.at[8])]
    wuc = [colcp(wu_hbm, wu_v, 0, F0, sem_c.at[9]), colcp(wu_hbm, wu_v, F0, FF - F0, sem_c.at[10])]
    ocp = [colcp(ob, o_hbm, j * BM, BM, sem_o.at[j]) for j in range(NB - 1)]
    ocp += [colcp(ob, o_hbm, (NB - 1) * BM + i * 256, 256, sem_o.at[NB - 1 + i]) for i in range(2)]

    rf_w, ci_w, fa_w, gs_w = _words(rf_v), _words(ci_v), _words(fa_v), _words(gs)
    ab_w, zt_w = _words(ab), _words(zt)
    ye_w, yo_w, ve_w, vo_w, se_w, so_w = (_words(r) for r in (ye, yo, ve, vo, se, so))
    hb_w, a2_w, a1_w = _words(hb), _words(a2), _words(a1)
    wg2_w, wu2_w, wg1_w, wu1_w = (_words(r) for r in (wg2, wu2, wg1, wu1))
    wds_w, hs_w = _words(wds), _words(hs)

    def ln1(t):
        xt = x_v[:, t * 128:(t + 1) * 128].astype(F32)
        a0 = xt[:H] + xt[H:]
        b0 = xt[:H] - xt[H:]
        yield
        m2 = jnp.sum(a0, axis=0, keepdims=True) * (2.0 / D)
        ca = a0 - m2
        yield
        v = jnp.sum(ca * ca + b0 * b0, axis=0, keepdims=True) * (0.5 / D)
        r = lax.rsqrt(v + EPS)
        yield
        ab[t, 0:H, :] = (ca * r).astype(BF)
        yield
        ab[t, H:D, :] = (b0 * r).astype(BF)

    def dfwd(t):
        for (e, dst) in ((0, ze), (1, zo)):
            lhs = jnp.concatenate([_bf(rf_w[0, e * 128:(e + 1) * 128, :]),
                                   _bf(rf_w[1, e * 128:(e + 1) * 128, :])[:, :H - 128]], axis=1)
            res = _nn(lhs, _bf(ab_w[t, e * (H // 2):(e + 1) * (H // 2), :]))
            zt[t, e] = res.astype(BF)
            yield
            w = zt_w[t, e].T
            for g in range(2):
                dst[pl.ds(PZ * (2 * t + g), N2), :] = w[N2 * g:N2 * (g + 1)]
            yield

    row8 = lax.broadcasted_iota(jnp.int32, (8, 128), 0)

    def wprep(t, src, dst):
        wd_ = pltpu.bitcast(src[0:H, t * 128:(t + 1) * 128], U32)
        ny = src[H:H + 1, t * 128:(t + 1) * 128].astype(F32)
        ny = pltpu.bitcast(jnp.broadcast_to(ny, (8, 128)), U32) >> 16
        ny = jnp.where(row8 == 0, ny, jnp.zeros_like(ny))
        wt = jnp.concatenate([wd_, ny, jnp.zeros((8, 128), U32)], axis=0).T
        for g in range(4):
            dst[pl.ds(PW * (4 * t + g), N1), :] = wt[N1 * g:N1 * (g + 1)]
        yield

    def gather2(src, s0, s1, pitch):
        return _bf(jnp.concatenate([src[pl.ds(s0, N1, stride=pitch), :],
                                    src[pl.ds(s1, N1, stride=pitch), :]], axis=0))

    def stage_a(ps):
        rhs = jnp.concatenate([gather2(z, p, p + N1, PZ) for p in ps for z in (ze, zo)], axis=1)
        res = _nn(_bf(fa_w[0]), rhs)
        i = 0
        for p in ps:
            for y in (ye, yo):
                y[pl.ds(2 * PY * p, 128), :] = res[:, i * 128:(i + 1) * 128].astype(BF)
                i += 1
        yield

    def stage_b(k1):
        g = (gt_v[0:128, :] * gt_v[256 + k1:257 + k1, :]
             + gt_v[128:256, :] * gt_v[288 + k1:289 + k1, :]).astype(BF)
        gs[k1] = g
        rhs = jnp.concatenate([gather2(y, k1, N1 + k1, PY) for y in (ye_w, yo_w)], axis=1)
        xx = _nn(g, rhs)
        xs[k1, 0] = xx[:, :128]
        xs[k1, 1] = xx[:, 128:]
        yield

    def stage_bi(k1):
        wr = wsr[pl.ds(k1, N2, stride=PW), :]
        wi = wsi[pl.ds(k1, N2, stride=PW), :]
        par = ((wr << 16, wi << 16),
               (wr & jnp.uint32(0xFFFF0000), wi & jnp.uint32(0xFFFF0000)))
        tiles = []
        for e in range(2):
            w_r, w_i = (pltpu.bitcast(w, F32) for w in par[e])
            x_r, x_i = xs[k1, e, 0:N2, :], xs[k1, e, N2:128, :]
            tiles.append(jnp.concatenate([x_r * w_r - x_i * w_i, x_r * w_i + x_i * w_r],
                                         axis=0).astype(BF))
        yy = _nn(_bf(gs_w[k1]).T, jnp.concatenate(tiles, axis=1))
        ve[pl.ds(2 * PY * k1, 128), :] = yy[:, :128].astype(BF)
        vo[pl.ds(2 * PY * k1, 128), :] = yy[:, 128:].astype(BF)
        yield

    def stage_ai(ps):
        rhs = jnp.concatenate([gather2(v, 2 * p, 2 * p + 1, PY) for p in ps for v in (ve_w, vo_w)],
                              axis=1)
        res = _nn(_bf(fa_w[1]), rhs)
        i = 0
        for p in ps:
            for y in (se, so):
                y[pl.ds(2 * PY * p, 128), :] = res[:, i * 128:(i + 1) * 128].astype(BF)
                i += 1
        yield

    def prep(j):
        b = j % 2
        for i in range(4):
            t = 4 * j + i

            def inv_d(e, src):
                rhs = jnp.concatenate(
                    [_bf(jnp.concatenate([src[pl.ds(ro * N1 + 2 * t + g, N1, stride=PY), :]
                                          for g in range(2)], axis=0))
                     for ro in range(2)], axis=1)
                lhs = jnp.concatenate([_bf(ci_w[2 * e]), _bf(ci_w[2 * e + 1])], axis=1)
                return _nt(lhs, rhs)
            ep = inv_d(0, se_w)
            op = inv_d(1, so_w)
            xt = x_v[:, t * 128:(t + 1) * 128].astype(F32)
            h = jnp.concatenate([xt[:H] + (ep + op), xt[H:] + (ep - op)], axis=0)
            hb[b, i] = h.astype(BF)
            m = jnp.mean(h, axis=0, keepdims=True)
            cen = h - m
            v = jnp.mean(cen * cen, axis=0, keepdims=True)
            cn[i] = cen * lax.rsqrt(v + EPS)
        blk = lambda mh, kh, ml, kl: cn[2 * mh + ml, Q * (2 * kh + kl):Q * (2 * kh + kl + 1), :]
        zpad = jnp.zeros((128 - Q, 128), F32)

        def put(dst_w, idx, v):
            dst_w[idx] = pltpu.bitcast(jnp.concatenate([v, zpad], axis=0).astype(BF).T, U32)

        for i in range(7):
            li = [[_term(TERMS_A[i], lambda q: blk(q // 2, q % 2, ml, kl)) for kl in range(2)]
                  for ml in range(2)]
            for ml in range(2):
                for kl in range(2):
                    put(a1_w, (b, i, ml, kl), li[ml][kl])
            ops = _seven_a(li[0][0], li[0][1], li[1][0], li[1][1])
            for k in range(7):
                put(a2_w, (b, 7 * i + k), ops[k])
        yield

    def wblk(w_v, kq, f0):
        return w_v[Q * kq:Q * (kq + 1), f0:f0 + 128].astype(F32)

    def store_hs(kt, pair, q11, q21, q12, q22):
        ops = _seven_b(q11, q21, q12, q22)
        for i in range(7):
            hs[i, kt, pair * 128:(pair + 1) * 128, :] = ops[i].astype(BF)

    def gate2(j, c):
        res = []
        for w_v, w2, w2_w in ((wg_v, wg2, wg2_w), (wu_v, wu2, wu2_w)):
            mm = []
            for i in range(7):
                if j == 0:
                    ri = [[_term(TERMS_B[i], lambda q: wblk(w_v, 2 * (q // 2) + kl,
                                                            512 * c + 128 * (2 * (q % 2) + fl)))
                           for fl in range(2)] for kl in range(2)]
                    ops = _seven_b(ri[0][0], ri[0][1], ri[1][0], ri[1][1])
                    for k in range(7):
                        w2[c, 7 * i + k] = ops[k].astype(BF)
                ops = [_bf(w2_w[c, 7 * i + k]) for k in range(7)]
                mm.append(_combine([_nn(_bf(a2_w[j % 2, 7 * i + k])[:, :Q], ops[k]) for k in range(7)]))
            res.append([_combine([mm[i][t] for i in range(7)]) for t in range(4)])
        q = [[res[0][t][o] * res[1][t][o] for o in range(4)] for t in range(4)]
        tile = lambda mt, ft: q[(mt % 2) * 2 + ft % 2][(mt // 2) * 2 + ft // 2]
        for fl in range(2):
            for ml in range(2):
                store_hs(2 * c + fl, ml, tile(ml, fl), tile(2 + ml, fl), tile(ml, 2 + fl), tile(2 + ml, 2 + fl))
        yield

    def gate1(j):
        res = []
        for w_v, w1, w1_w in ((wg_v, wg1, wg1_w), (wu_v, wu1, wu1_w)):
            if j == 0:
                for kl in range(2):
                    ops = _seven_b(wblk(w_v, kl, F1), wblk(w_v, kl, F1 + 128),
                                   wblk(w_v, 2 + kl, F1), wblk(w_v, 2 + kl, F1 + 128))
                    for i in range(7):
                        w1[i, kl] = ops[i].astype(BF)
            ops = [[_bf(w1_w[i, kl]) for i in range(7)] for kl in range(2)]
            m = []
            for i in range(7):
                part = [_nn(jnp.concatenate([_bf(a1_w[j % 2, i, ml, kl])[:, :Q] for ml in range(2)], axis=0),
                            ops[kl][i]) for kl in range(2)]
                m.append(part[0] + part[1])
            res.append(_combine(m))
        q11, q12, q21, q22 = [g_ * u_ for g_, u_ in zip(*res)]
        for ml in range(2):
            sl = slice(128 * ml, 128 * (ml + 1))
            store_hs(NKT - 1, ml, q11[sl], q21[sl], q12[sl], q22[sl])
        yield

    def wd_cols(kt, fh):
        if kt < 2 * NC2:
            return 512 * (kt // 2) + 128 * (kt % 2) + 256 * fh
        return F1 + 128 * fh

    def down(j):
        if j == 0:
            quad = lambda kt, d, fh: wd_v[H * d:H * (d + 1), wd_cols(kt, fh):wd_cols(kt, fh) + 128].astype(F32)
            for kt in range(NKT):
                ops = _seven_a(quad(kt, 0, 0), quad(kt, 0, 1), quad(kt, 1, 0), quad(kt, 1, 1))
                for i in range(7):
                    wds[i, kt] = ops[i].astype(BF)
        ops = [[_bf(wds_w[i, kt]) for i in range(7)] for kt in range(NKT)]
        m = []
        for i in range(7):
            lhs = jnp.concatenate([ops[kt][i] for kt in range(NKT)], axis=1)
            rhs = jnp.concatenate([_bf(hs_w[i, kt]) for kt in range(NKT)], axis=1)
            m.append(_nt(lhs, rhs))
        o11, o12, o21, o22 = _combine(m)
        for mh, (lo, hi) in enumerate(((o11, o21), (o12, o22))):
            for ml in range(2):
                i = 2 * mh + ml
                t = 4 * j + i
                sl = slice(128 * ml, 128 * (ml + 1))
                hh_ = _bf(hb_w[j % 2, i]).astype(F32)
                ob[0:H, t * 128:(t + 1) * 128] = (hh_[:H] + lo[:, sl]).astype(BF)
                ob[H:D, t * 128:(t + 1) * 128] = (hh_[H:] + hi[:, sl]).astype(BF)
            if j == NB - 1:
                ocp[j + mh].start()
        if j < NB - 1:
            ocp[j].start()
        yield

    for c in (xcp[0], c_rf, *xcp[1:], c_fa, c_wr, c_gt, c_wi, c_ci,
              wgc[0], wuc[0], wgc[1], wuc[1], c_wd):
        c.start()
        pl.semaphore_signal(sem_f, 1)
        pl.semaphore_wait(sem_f, 1)
    for c in range(NXC):
        xcp[c].wait()
        if c == 0:
            seed = x_v[0:8, 0:128]
            for buf in (ab, zt, gs, hb, a2, a1, wg2, wu2, wg1, wu1, wds, hs):
                buf[(0,) * (len(buf.shape) - 2) + (slice(0, 8), slice(None))] = seed
            xs[0, 0, 0:1, :] = seed[0:1].astype(F32)
            cn[0, 0:1, :] = seed[0:1].astype(F32)
            for t in range(XT[0], XT[1]):
                _run(ln1(t))
            c_rf.wait()
        for t in range(XT[c], XT[c + 1]):
            if c > 0:
                _run(ln1(t))
            _run(dfwd(t))
    NG = N1 // 2
    c_fa.wait()
    _run(_seq(*[stage_a([2 * g, 2 * g + 1]) for g in range(NG // 2)]))
    c_wr.wait()
    _run(_mix(_seq(*[stage_a([2 * g, 2 * g + 1]) for g in range(NG // 2, NG)]), NG // 2,
              _seq(*[wprep(t, wr_v, wsr) for t in range(NT)]), NT))
    c_gt.wait()
    _run(_seq(*[stage_b(k1) for k1 in range(N1 // 2)]))
    c_wi.wait()
    _run(_mix(_seq(*[stage_b(k1) for k1 in range(N1 // 2, N1)]), N1 // 2,
              _seq(*[wprep(t, wi_v, wsi) for t in range(NT)]), NT))
    for k1 in range(N1):
        _run(stage_bi(k1))
    for g in range(NG):
        _run(stage_ai([2 * g, 2 * g + 1]))
    c_ci.wait()
    wgc[0].wait()
    wuc[0].wait()
    _run(prep(0))
    for j in range(NB):
        nxt = prep(j + 1) if j + 1 < NB else _seq()
        if j == 0:
            _run(_rr(_seq(gate2(0, 0), gate2(0, 1)), nxt))
            wgc[1].wait()
            wuc[1].wait()
            c_wd.wait()
            _run(_seq(gate2(0, 2), gate1(0), down(0)))
        else:
            _run(_rr(_seq(*[gate2(j, c) for c in range(NC2)], gate1(j), down(j)), nxt))
    for c in ocp:
        c.wait()


def _skip(n):
    for _ in range(n):
        yield


@jax.jit
def pallas_sequential_preLN__spectral_gfnet__glu_gated_bilinear__prompt_kernel(
    A_x, A_w_r, A_w_i, B_x, B_w_gate, B_w_up, B_w_down,
):
    del B_x
    xT = jnp.transpose(A_x.reshape(S, D))
    any_spec = pl.BlockSpec(memory_space=pl.ANY)
    vm = pltpu.VMEM
    dma = pltpu.SemaphoreType.DMA
    slab = vm((2 * PY * N1, 128), BF)
    oT = pl.pallas_call(
        _kernel,
        out_shape=jax.ShapeDtypeStruct((D, S), BF),
        in_specs=[any_spec] * 10,
        out_specs=any_spec,
        scratch_shapes=[
            vm((D, S), BF), vm((H + 1, S), BF), vm((H + 1, S), BF),
            vm((D, FF), BF), vm((D, FF), BF), vm((D, FF), BF),
            vm(_RF.shape, BF), vm(_CI.shape, BF), vm(_FA.shape, BF), vm(_GT.shape, F32),
            vm((N1, 128, 128), BF), vm((N1, 2, 128, 128), F32),
            vm((NT, D, 128), BF), vm((NT, 2, 256, 128), BF),
            vm((N1 * PZ, 128), U32), vm((N1 * PZ, 128), U32),
            slab, slab, slab, slab,
            vm((N2 * PW, 128), U32), vm((N2 * PW, 128), U32),
            slab, slab,
            vm((2, 4, D, 128), BF), vm((4, D, 128), F32),
            vm((2, 49, 128, 128), BF), vm((2, 7, 2, 2, 128, 128), BF),
            vm((NC2, 49, Q, 128), BF), vm((NC2, 49, Q, 128), BF),
            vm((7, 2, Q, 128), BF), vm((7, 2, Q, 128), BF),
            vm((7, NKT, H, 128), BF), vm((7, NKT, 256, 128), BF), vm((D, S), BF),
            dma((NXC,)), dma((11,)), dma((NB + 1,)), pltpu.SemaphoreType.REGULAR,
        ],
        compiler_params=pltpu.CompilerParams(vmem_limit_bytes=100 * 1024 * 1024),
        name="gfnet_glu",
    )(xT, A_w_r.T, A_w_i.T, B_w_gate, B_w_up, B_w_down.T, _RF, _CI, _FA, _GT)
    return jnp.transpose(oT).reshape(1, S, D)
```

```python
import numpy as np
import jax
import jax.numpy as jnp
from jax import lax
from jax.experimental import pallas as pl
from jax.experimental.pallas import tpu as pltpu

S, D, FF = 2048, 448, 1792
H = D // 2
N1, N2 = 32, 64
PZ = N2 + 1
PW = N1 + 1
PY = N2 + 4
BF = jnp.bfloat16
F32 = jnp.float32
U32 = jnp.uint32
EPS = 1e-5


def _consts():
    d = np.arange(H)
    rf = np.zeros((512, 256))
    for m in range(H // 2 + 1):
        ang = -2.0 * np.pi * ((2 * m * d) % D) / D
        rf[2 * m, :H] = np.cos(ang)
        rf[2 * m + 1, :H] = np.sin(ang)
    for m in range(H // 2):
        ang = -2.0 * np.pi * (((2 * m + 1) * d) % D) / D
        rf[256 + 2 * m, :H] = np.cos(ang)
        rf[256 + 2 * m + 1, :H] = np.sin(ang)
    ci = np.zeros((2, H, 256))
    for m in range(H // 2 + 1):
        k = 2 * m
        c = 1.0 if (k == 0 or k == H) else 2.0
        ang = 2.0 * np.pi * ((k * d) % D) / D
        ci[0, :, m] = c * np.cos(ang) / (S * D)
        if k != 0 and k != H:
            ci[0, :, 128 + m] = -c * np.sin(ang) / (S * D)
    for m in range(H // 2):
        k = 2 * m + 1
        ang = 2.0 * np.pi * ((k * d) % D) / D
        ci[1, :, m] = 2.0 * np.cos(ang) / (S * D)
        ci[1, :, 128 + m] = -2.0 * np.sin(ang) / (S * D)
    n1 = np.arange(N1)
    n2 = np.arange(N2)
    ang = -2.0 * np.pi * ((np.outer(n1, n1)) % N1) / N1
    fr, fi = np.cos(ang), np.sin(ang)
    fa = np.zeros((2, 128, 128))
    for mu in range(2):
        o = 64 * mu
        fa[0, o + 0:o + 64:2, o + 0:o + 64:2] = fr
        fa[0, o + 0:o + 64:2, o + 1:o + 64:2] = -fi
        fa[0, o + 1:o + 64:2, o + 0:o + 64:2] = fi
        fa[0, o + 1:o + 64:2, o + 1:o + 64:2] = fr
        fa[1, mu:64:2, o + 0:o + 64:2] = fr
        fa[1, mu:64:2, o + 1:o + 64:2] = fi
        fa[1, 64 + mu:128:2, o + 0:o + 64:2] = -fi
        fa[1, 64 + mu:128:2, o + 1:o + 64:2] = fr
    ang = -2.0 * np.pi * (np.outer(n2, n2) % N2) / N2
    fr, fi = np.cos(ang), np.sin(ang)
    pq = np.zeros((2, 128, 128))
    pq[0, 0:64, 0::2], pq[1, 0:64, 0::2] = fr, -fi
    pq[0, 0:64, 1::2], pq[1, 0:64, 1::2] = -fi, -fr
    pq[0, 64:128, 0::2], pq[1, 64:128, 0::2] = fi, fr
    pq[0, 64:128, 1::2], pq[1, 64:128, 1::2] = fr, -fi
    ang = -2.0 * np.pi * np.outer(n1, n2) / S
    tw = np.stack([np.repeat(np.cos(ang), 2, axis=1), np.repeat(np.sin(ang), 2, axis=1)])
    gt = np.concatenate([pq.reshape(256, 128), tw.reshape(64, 128)]).astype(np.float32)
    tb = lambda a: np.asarray(a, dtype=np.float32).astype(BF)
    rf = np.stack([rf[:, :128], rf[:, 128:]])
    ci = np.stack([ci[0, :, :128], ci[0, :, 128:], ci[1, :, :128], ci[1, :, 128:]])
    return tb(rf), tb(ci), tb(fa), gt


_RF, _CI, _FA, _GT = _consts()


def _nn(a, b):
    return jnp.dot(a, b, preferred_element_type=F32)


def _nt(a, b):
    return lax.dot_general(a, b, (((1,), (1,)), ((), ())), preferred_element_type=F32)


def _tn(a, b):
    return lax.dot_general(a, b, (((0,), (0,)), ((), ())), preferred_element_type=F32)


def _run(g):
    for _ in g:
        pass


def _seq(*gs):
    for g in gs:
        yield from g


def _rr(*gs):
    gs = list(gs)
    while gs:
        nxt = []
        for g in gs:
            try:
                next(g)
                nxt.append(g)
            except StopIteration:
                pass
        gs = nxt
        yield


NT = S // 128
XT = (0, 4, 8, 16)
NXC = len(XT) - 1
BM = 512
NB = S // BM
Q = D // 4
NC2 = 3
F1 = 512 * NC2
RC = 32
RP = 16
F0 = 1024
NKT = FF // 256


def _take(g, n):
    for _ in range(n):
        try:
            next(g)
        except StopIteration:
            return
        yield


def _mix(ga, na, gb, nb):
    k = 0
    for a in range(na):
        next(ga, None)
        while k < (a + 1) * nb // na:
            next(gb, None)
            k += 1
        yield
    _run(ga)
    _run(gb)


def _seven_b(b11, b12, b21, b22):
    return (b11 + b22, b11, b12 - b22, b21 - b11, b22, b11 + b12, b21 + b22)


def _seven_a(a11, a12, a21, a22):
    return (a11 + a22, a21 + a22, a11, a22, a11 + a12, a21 - a11, a12 - a22)


TERMS_A = (((1, 0), (1, 3)), ((1, 2), (1, 3)), ((1, 0),), ((1, 3),),
           ((1, 0), (1, 1)), ((1, 2), (-1, 0)), ((1, 1), (-1, 3)))
TERMS_B = (((1, 0), (1, 3)), ((1, 0),), ((1, 1), (-1, 3)), ((1, 2), (-1, 0)),
           ((1, 3),), ((1, 0), (1, 1)), ((1, 2), (1, 3)))


def _term(terms, get):
    v = get(terms[0][1])
    for sign, q in terms[1:]:
        v = v + get(q) if sign > 0 else v - get(q)
    return v


def _fold8(v):
    parts = [v[r:r + 8] for r in range(0, v.shape[0], 8)]
    while len(parts) > 1:
        parts = [parts[k] + parts[k + 1] if k + 1 < len(parts) else parts[k]
                 for k in range(0, len(parts), 2)]
    return parts[0]


def _combine(m):
    return (m[0] + m[3] - m[4] + m[6], m[2] + m[4], m[1] + m[3], m[0] - m[1] + m[2] + m[5])


def _words(ref):
    return ref.bitcast(U32)


def _bf(w):
    return pltpu.bitcast(w, BF)


def _kernel(x_hbm, wr_hbm, wi_hbm, wg_hbm, wu_hbm, wd_hbm,
            rf_hbm, ci_hbm, fa_hbm, gt_hbm,
            o_hbm,
            x_v, wr_v, wi_v, wg_v, wu_v, wd_v,
            rf_v, ci_v, fa_v, gt_v, gs, xs,
            ab, zt, ze, zo, ye, yo, ve, vo, wsr, wsi, se, so,
            hb, cn, a2, a1, wg2, wu2, wg1, wu1, wds, hs, ob,
            sem_x, sem_c, sem_o, sem_f):

    def colcp(src, dst, c0, w, sem):
        return pltpu.make_async_copy(src.at[:, pl.ds(c0, w)], dst.at[:, pl.ds(c0, w)], sem)

    xcp = [colcp(x_hbm, x_v, XT[c] * 128, (XT[c + 1] - XT[c]) * 128, sem_x.at[c])
           for c in range(NXC)]
    c_rf = pltpu.make_async_copy(rf_hbm, rf_v, sem_c.at[0])
    c_fa = pltpu.make_async_copy(fa_hbm, fa_v, sem_c.at[1])
    c_ci = pltpu.make_async_copy(ci_hbm, ci_v, sem_c.at[2])
    c_wr = pltpu.make_async_copy(wr_hbm, wr_v, sem_c.at[3])
    c_wi = pltpu.make_async_copy(wi_hbm, wi_v, sem_c.at[4])
    c_gt = pltpu.make_async_copy(gt_hbm, gt_v, sem_c.at[5])
    c_wd = pltpu.make_async_copy(wd_hbm, wd_v, sem_c.at[6])
    wgc = [colcp(wg_hbm, wg_v, 0, F0, sem_c.at[7]), colcp(wg_hbm, wg_v, F0, FF - F0, sem_c.at[8])]
    wuc = [colcp(wu_hbm, wu_v, 0, F0, sem_c.at[9]), colcp(wu_hbm, wu_v, F0, FF - F0, sem_c.at[10])]
    ocp = [colcp(ob, o_hbm, j * BM, BM, sem_o.at[j]) for j in range(NB - 1)]
    ocp += [colcp(ob, o_hbm, (NB - 1) * BM + i * 256, 256, sem_o.at[NB - 1 + i]) for i in range(2)]

    rf_w, ci_w, fa_w, gs_w = _words(rf_v), _words(ci_v), _words(fa_v), _words(gs)
    ab_w, zt_w = _words(ab), _words(zt)
    ye_w, yo_w, ve_w, vo_w, se_w, so_w = (_words(r) for r in (ye, yo, ve, vo, se, so))
    hb_w, a2_w, a1_w = _words(hb), _words(a2), _words(a1)
    wg2_w, wu2_w, wg1_w, wu1_w = (_words(r) for r in (wg2, wu2, wg1, wu1))
    wds_w, hs_w = _words(wds), _words(hs)

    def ln1(t):
        xt = x_v[:, t * 128:(t + 1) * 128].astype(F32)
        a0 = xt[:H] + xt[H:]
        b0 = xt[:H] - xt[H:]
        yield
        m2 = jnp.sum(a0, axis=0, keepdims=True) * (2.0 / D)
        ca = a0 - m2
        yield
        v = jnp.sum(ca * ca + b0 * b0, axis=0, keepdims=True) * (0.5 / D)
        r = lax.rsqrt(v + EPS)
        yield
        ab[t, 0:H, :] = (ca * r).astype(BF)
        yield
        ab[t, H:D, :] = (b0 * r).astype(BF)

    def dfwd(t):
        for (e, dst) in ((0, ze), (1, zo)):
            lhs = jnp.concatenate([_bf(rf_w[0, e * 128:(e + 1) * 128, :]),
                                   _bf(rf_w[1, e * 128:(e + 1) * 128, :])[:, :H - 128]], axis=1)
            res = _nn(lhs, _bf(ab_w[t, e * (H // 2):(e + 1) * (H // 2), :]))
            zt[t, e] = res.astype(BF)
            yield
            w = zt_w[t, e].T
            for g in range(2):
                dst[pl.ds(PZ * (2 * t + g), N2), :] = w[N2 * g:N2 * (g + 1)]
            yield

    row8 = lax.broadcasted_iota(jnp.int32, (8, 128), 0)

    def wprep(t, src, dst):
        wd_ = pltpu.bitcast(src[0:H, t * 128:(t + 1) * 128], U32)
        ny = src[H:H + 1, t * 128:(t + 1) * 128].astype(F32)
        ny = pltpu.bitcast(jnp.broadcast_to(ny, (8, 128)), U32) >> 16
        ny = jnp.where(row8 == 0, ny, jnp.zeros_like(ny))
        wt = jnp.concatenate([wd_, ny, jnp.zeros((8, 128), U32)], axis=0).T
        for g in range(4):
            dst[pl.ds(PW * (4 * t + g), N1), :] = wt[N1 * g:N1 * (g + 1)]
        yield

    def gather2(src, s0, s1, pitch):
        return _bf(jnp.concatenate([src[pl.ds(s0, N1, stride=pitch), :],
                                    src[pl.ds(s1, N1, stride=pitch), :]], axis=0))

    def stage_a(ps):
        rhs = jnp.concatenate([gather2(z, p, p + N1, PZ) for p in ps for z in (ze, zo)], axis=1)
        res = _nn(_bf(fa_w[0]), rhs)
        i = 0
        for p in ps:
            for y in (ye, yo):
                y[pl.ds(2 * PY * p, 128), :] = res[:, i * 128:(i + 1) * 128].astype(BF)
                i += 1
        yield

    def stage_b(k1):
        g = (gt_v[0:128, :] * gt_v[256 + k1:257 + k1, :]
             + gt_v[128:256, :] * gt_v[288 + k1:289 + k1, :]).astype(BF)
        gs[k1] = g
        rhs = jnp.concatenate([gather2(y, k1, N1 + k1, PY) for y in (ye_w, yo_w)], axis=1)
        xx = _nn(g, rhs)
        xs[k1, 0] = xx[:, :128]
        xs[k1, 1] = xx[:, 128:]
        yield

    def stage_bi(k1):
        wr = wsr[pl.ds(k1, N2, stride=PW), :]
        wi = wsi[pl.ds(k1, N2, stride=PW), :]
        par = ((wr << 16, wi << 16),
               (wr & jnp.uint32(0xFFFF0000), wi & jnp.uint32(0xFFFF0000)))
        tiles = []
        for e in range(2):
            w_r, w_i = (pltpu.bitcast(w, F32) for w in par[e])
            x_r, x_i = xs[k1, e, 0:N2, :], xs[k1, e, N2:128, :]
            tiles.append(jnp.concatenate([x_r * w_r - x_i * w_i, x_r * w_i + x_i * w_r],
                                         axis=0).astype(BF))
        yy = _nn(_bf(gs_w[k1]).T, jnp.concatenate(tiles, axis=1))
        ve[pl.ds(2 * PY * k1, 128), :] = yy[:, :128].astype(BF)
        vo[pl.ds(2 * PY * k1, 128), :] = yy[:, 128:].astype(BF)
        yield

    def stage_ai(ps):
        rhs = jnp.concatenate([gather2(v, 2 * p, 2 * p + 1, PY) for p in ps for v in (ve_w, vo_w)],
                              axis=1)
        res = _nn(_bf(fa_w[1]), rhs)
        i = 0
        for p in ps:
            for y in (se, so):
                y[pl.ds(2 * PY * p, 128), :] = res[:, i * 128:(i + 1) * 128].astype(BF)
                i += 1
        yield

    def prep_tiles(j, tiles):
        def inv_d(e, src):
            rhs = jnp.concatenate(
                [jnp.concatenate(
                    [_bf(jnp.concatenate([src[pl.ds(ro * N1 + 2 * (4 * j + i) + g, N1, stride=PY), :]
                                          for g in range(2)], axis=0))
                     for ro in range(2)], axis=1) for i in tiles], axis=0)
            lhs = jnp.concatenate([_bf(ci_w[2 * e]), _bf(ci_w[2 * e + 1])], axis=1)
            return _nt(lhs, rhs)
        ep = inv_d(0, se_w)
        op = inv_d(1, so_w)
        for n, i in enumerate(tiles):
            t = 4 * j + i
            cols = slice(128 * n, 128 * (n + 1))
            acc = None
            for r in range(0, H, RC):
                e, o = ep[r:r + RC, cols], op[r:r + RC, cols]
                lo = x_v[r:r + RC, t * 128:(t + 1) * 128].astype(F32) + (e + o)
                hi = x_v[H + r:H + r + RC, t * 128:(t + 1) * 128].astype(F32) + (e - o)
                for r0, v in ((r, lo), (H + r, hi)):
                    hb[j % 2, i, r0:r0 + RC, :] = v.astype(BF)
                    cn[i, r0:r0 + RC, :] = v
                part = _fold8(lo + hi)
                acc = part if acc is None else acc + part
            m = jnp.sum(acc, axis=0, keepdims=True) * (1.0 / D)
            acc = None
            for r in range(0, D, 2 * RC):
                c = cn[i, r:r + 2 * RC, :] - m
                part = _fold8(c * c)
                acc = part if acc is None else acc + part
            rs = lax.rsqrt(jnp.sum(acc, axis=0, keepdims=True) * (1.0 / D) + EPS)
            for r in range(0, D, 2 * RC):
                cn[i, r:r + 2 * RC, :] = (cn[i, r:r + 2 * RC, :] - m) * rs

    def prep_ops():
        blk = lambda mh, kh, ml, kl: cn[2 * mh + ml, Q * (2 * kh + kl):Q * (2 * kh + kl + 1), :]
        zpad = jnp.zeros((128 - Q, 128), F32)

        def put(dst_w, idx, v):
            dst_w[idx] = pltpu.bitcast(jnp.concatenate([v, zpad], axis=0).astype(BF).T, U32)

        def lvl1(i, ml, kl):
            return _term(TERMS_A[i], lambda q: blk(q // 2, q % 2, ml, kl))

        for i in range(7):
            for ml in range(2):
                for kl in range(2):
                    put(a1_w, (i, ml, kl), lvl1(i, ml, kl))
            for k in range(7):
                put(a2_w, (7 * i + k,), _term(TERMS_A[k], lambda q: lvl1(i, q // 2, q % 2)))

    def wblk(w_v, kq, f0, r):
        return w_v[Q * kq + r:Q * kq + r + RP, f0:f0 + 128].astype(F32)

    def store_hs(kt, pair, q11, q21, q12, q22):
        ops = _seven_b(q11, q21, q12, q22)
        for i in range(7):
            hs[i, kt, pair * 128:(pair + 1) * 128, :] = ops[i].astype(BF)

    def gate2(j, c):
        res = []
        for w_v, w2, w2_w in ((wg_v, wg2, wg2_w), (wu_v, wu2, wu2_w)):
            mm = []
            for i in range(7):
                if j == 0:
                    for r in range(0, Q, RP):
                        ri = [[_term(TERMS_B[i], lambda q: wblk(w_v, 2 * (q // 2) + kl,
                                                                512 * c + 128 * (2 * (q % 2) + fl), r))
                               for fl in range(2)] for kl in range(2)]
                        ops = _seven_b(ri[0][0], ri[0][1], ri[1][0], ri[1][1])
                        for k in range(7):
                            w2[c, 7 * i + k, r:r + RP, :] = ops[k].astype(BF)
                ops = [_bf(w2_w[c, 7 * i + k]) for k in range(7)]
                mm.append(_combine([_nn(_bf(a2_w[7 * i + k])[:, :Q], ops[k]) for k in range(7)]))
                yield
            res.append([_combine([mm[i][t] for i in range(7)]) for t in range(4)])
        q = [[res[0][t][o] * res[1][t][o] for o in range(4)] for t in range(4)]
        tile = lambda mt, ft: q[(mt % 2) * 2 + ft % 2][(mt // 2) * 2 + ft // 2]
        for fl in range(2):
            for ml in range(2):
                store_hs(2 * c + fl, ml, tile(ml, fl), tile(2 + ml, fl), tile(ml, 2 + fl), tile(2 + ml, 2 + fl))
        yield

    def gate1(j):
        res = []
        for w_v, w1, w1_w in ((wg_v, wg1, wg1_w), (wu_v, wu1, wu1_w)):
            if j == 0:
                for kl in range(2):
                    for r in range(0, Q, RP):
                        ops = _seven_b(wblk(w_v, kl, F1, r), wblk(w_v, kl, F1 + 128, r),
                                       wblk(w_v, 2 + kl, F1, r), wblk(w_v, 2 + kl, F1 + 128, r))
                        for i in range(7):
                            w1[i, kl, r:r + RP, :] = ops[i].astype(BF)
            ops = [[_bf(w1_w[i, kl]) for i in range(7)] for kl in range(2)]
            m = []
            for i in range(7):
                part = [_nn(jnp.concatenate([_bf(a1_w[i, ml, kl])[:, :Q] for ml in range(2)], axis=0),
                            ops[kl][i]) for kl in range(2)]
                m.append(part[0] + part[1])
            res.append(_combine(m))
        q11, q12, q21, q22 = [g_ * u_ for g_, u_ in zip(*res)]
        for ml in range(2):
            sl = slice(128 * ml, 128 * (ml + 1))
            store_hs(NKT - 1, ml, q11[sl], q21[sl], q12[sl], q22[sl])
        yield

    def wd_cols(kt, fh):
        if kt < 2 * NC2:
            return 512 * (kt // 2) + 128 * (kt % 2) + 256 * fh
        return F1 + 128 * fh

    def down(j):
        if j == 0:
            for kt in range(NKT):
                for r in range(0, H, 2 * RP):
                    quad = lambda d, fh: wd_v[H * d + r:H * d + r + 2 * RP,
                                              wd_cols(kt, fh):wd_cols(kt, fh) + 128].astype(F32)
                    ops = _seven_a(quad(0, 0), quad(0, 1), quad(1, 0), quad(1, 1))
                    for i in range(7):
                        wds[i, kt, r:r + 2 * RP, :] = ops[i].astype(BF)
        ops = [[_bf(wds_w[i, kt]) for i in range(7)] for kt in range(NKT)]
        m = []
        for i in range(7):
            lhs = jnp.concatenate([ops[kt][i] for kt in range(NKT)], axis=1)
            rhs = jnp.concatenate([_bf(hs_w[i, kt]) for kt in range(NKT)], axis=1)
            m.append(_nt(lhs, rhs))
            yield
        o11, o12, o21, o22 = _combine(m)
        for mh, (lo, hi) in enumerate(((o11, o21), (o12, o22))):
            for ml in range(2):
                i = 2 * mh + ml
                t = 4 * j + i
                sl = slice(128 * ml, 128 * (ml + 1))
                hh_ = _bf(hb_w[j % 2, i]).astype(F32)
                ob[0:H, t * 128:(t + 1) * 128] = (hh_[:H] + lo[:, sl]).astype(BF)
                ob[H:D, t * 128:(t + 1) * 128] = (hh_[H:] + hi[:, sl]).astype(BF)
            if j == NB - 1:
                ocp[j + mh].start()
        if j < NB - 1:
            ocp[j].start()
        yield

    for c in (xcp[0], c_rf, *xcp[1:], c_fa, c_wr, c_gt, c_wi, c_ci,
              wgc[0], wuc[0], wgc[1], wuc[1], c_wd):
        c.start()
        pl.semaphore_signal(sem_f, 1)
        pl.semaphore_wait(sem_f, 1)
    for c in range(NXC):
        xcp[c].wait()
        if c == 0:
            seed = x_v[0:8, 0:128]
            for buf in (ab, zt, gs, hb, a2, a1, wg2, wu2, wg1, wu1, wds, hs):
                buf[(0,) * (len(buf.shape) - 2) + (slice(0, 8), slice(None))] = seed
            xs[0, 0, 0:1, :] = seed[0:1].astype(F32)
            cn[0, 0:1, :] = seed[0:1].astype(F32)
            for t in range(XT[0], XT[1]):
                _run(ln1(t))
            c_rf.wait()
        for t in range(XT[c], XT[c + 1]):
            if c > 0:
                _run(ln1(t))
            _run(dfwd(t))
    NG = N1 // 2
    c_fa.wait()
    _run(_seq(*[stage_a([2 * g, 2 * g + 1]) for g in range(NG // 2)]))
    c_wr.wait()
    _run(_mix(_seq(*[stage_a([2 * g, 2 * g + 1]) for g in range(NG // 2, NG)]), NG // 2,
              _seq(*[wprep(t, wr_v, wsr) for t in range(NT)]), NT))
    c_gt.wait()
    _run(_seq(*[stage_b(k1) for k1 in range(N1 // 2)]))
    c_wi.wait()
    _run(_mix(_seq(*[stage_b(k1) for k1 in range(N1 // 2, N1)]), N1 // 2,
              _seq(*[wprep(t, wi_v, wsi) for t in range(NT)]), NT))
    for k1 in range(N1):
        _run(stage_bi(k1))
    for g in range(NG):
        _run(stage_ai([2 * g, 2 * g + 1]))
    c_ci.wait()
    wgc[0].wait()
    wuc[0].wait()
    for i in range(4):
        prep_tiles(0, (i,))
    prep_ops()
    for j in range(NB):
        for c in range(NC2 + 1):
            if j == 0 and c == 2:
                wgc[1].wait()
                wuc[1].wait()
                c_wd.wait()
            _run(gate2(j, c) if c < NC2 else gate1(j))
        for n, _ in enumerate(down(j)):
            if j + 1 < NB and n < 4:
                prep_tiles(j + 1, (n,))
            if j + 1 < NB and n == 4:
                prep_ops()
    for c in ocp:
        c.wait()


def _skip(n):
    for _ in range(n):
        yield


@jax.jit
def pallas_sequential_preLN__spectral_gfnet__glu_gated_bilinear__prompt_kernel(
    A_x, A_w_r, A_w_i, B_x, B_w_gate, B_w_up, B_w_down,
):
    del B_x
    xT = jnp.transpose(A_x.reshape(S, D))
    any_spec = pl.BlockSpec(memory_space=pl.ANY)
    vm = pltpu.VMEM
    dma = pltpu.SemaphoreType.DMA
    slab = vm((2 * PY * N1, 128), BF)
    oT = pl.pallas_call(
        _kernel,
        out_shape=jax.ShapeDtypeStruct((D, S), BF),
        in_specs=[any_spec] * 10,
        out_specs=any_spec,
        scratch_shapes=[
            vm((D, S), BF), vm((H + 1, S), BF), vm((H + 1, S), BF),
            vm((D, FF), BF), vm((D, FF), BF), vm((D, FF), BF),
            vm(_RF.shape, BF), vm(_CI.shape, BF), vm(_FA.shape, BF), vm(_GT.shape, F32),
            vm((N1, 128, 128), BF), vm((N1, 2, 128, 128), F32),
            vm((NT, D, 128), BF), vm((NT, 2, 256, 128), BF),
            vm((N1 * PZ, 128), U32), vm((N1 * PZ, 128), U32),
            slab, slab, slab, slab,
            vm((N2 * PW, 128), U32), vm((N2 * PW, 128), U32),
            slab, slab,
            vm((2, 4, D, 128), BF), vm((4, D, 128), F32),
            vm((49, 128, 128), BF), vm((7, 2, 2, 128, 128), BF),
            vm((NC2, 49, Q, 128), BF), vm((NC2, 49, Q, 128), BF),
            vm((7, 2, Q, 128), BF), vm((7, 2, Q, 128), BF),
            vm((7, NKT, H, 128), BF), vm((7, NKT, 256, 128), BF), vm((D, S), BF),
            dma((NXC,)), dma((11,)), dma((NB + 1,)), pltpu.SemaphoreType.REGULAR,
        ],
        compiler_params=pltpu.CompilerParams(vmem_limit_bytes=100 * 1024 * 1024),
        name="gfnet_glu",
    )(xT, A_w_r.T, A_w_i.T, B_w_gate, B_w_up, B_w_down.T, _RF, _CI, _FA, _GT)
    return jnp.transpose(oT).reshape(1, S, D)
```

```python
import numpy as np
import jax
import jax.numpy as jnp
from jax import lax
from jax.experimental import pallas as pl
from jax.experimental.pallas import tpu as pltpu

S, D, FF = 2048, 448, 1792
H = D // 2
N1, N2 = 32, 64
PZ = N2 + 1
PW = N1 + 1
PY = N2 + 4
BF = jnp.bfloat16
F32 = jnp.float32
U32 = jnp.uint32
EPS = 1e-5


def _consts():
    d = np.arange(H)
    rf = np.zeros((512, 256))
    for m in range(H // 2 + 1):
        ang = -2.0 * np.pi * ((2 * m * d) % D) / D
        rf[2 * m, :H] = np.cos(ang)
        rf[2 * m + 1, :H] = np.sin(ang)
    for m in range(H // 2):
        ang = -2.0 * np.pi * (((2 * m + 1) * d) % D) / D
        rf[256 + 2 * m, :H] = np.cos(ang)
        rf[256 + 2 * m + 1, :H] = np.sin(ang)
    ci = np.zeros((2, H, 256))
    for m in range(H // 2 + 1):
        k = 2 * m
        c = 1.0 if (k == 0 or k == H) else 2.0
        ang = 2.0 * np.pi * ((k * d) % D) / D
        ci[0, :, m] = c * np.cos(ang) / (S * D)
        if k != 0 and k != H:
            ci[0, :, 128 + m] = -c * np.sin(ang) / (S * D)
    for m in range(H // 2):
        k = 2 * m + 1
        ang = 2.0 * np.pi * ((k * d) % D) / D
        ci[1, :, m] = 2.0 * np.cos(ang) / (S * D)
        ci[1, :, 128 + m] = -2.0 * np.sin(ang) / (S * D)
    n1 = np.arange(N1)
    n2 = np.arange(N2)
    ang = -2.0 * np.pi * ((np.outer(n1, n1)) % N1) / N1
    fr, fi = np.cos(ang), np.sin(ang)
    fa = np.zeros((2, 128, 128))
    for mu in range(2):
        o = 64 * mu
        fa[0, o + 0:o + 64:2, o + 0:o + 64:2] = fr
        fa[0, o + 0:o + 64:2, o + 1:o + 64:2] = -fi
        fa[0, o + 1:o + 64:2, o + 0:o + 64:2] = fi
        fa[0, o + 1:o + 64:2, o + 1:o + 64:2] = fr
        fa[1, mu:64:2, o + 0:o + 64:2] = fr
        fa[1, mu:64:2, o + 1:o + 64:2] = fi
        fa[1, 64 + mu:128:2, o + 0:o + 64:2] = -fi
        fa[1, 64 + mu:128:2, o + 1:o + 64:2] = fr
    ang = -2.0 * np.pi * (np.outer(n2, n2) % N2) / N2
    fr, fi = np.cos(ang), np.sin(ang)
    pq = np.zeros((2, 128, 128))
    pq[0, 0:64, 0::2], pq[1, 0:64, 0::2] = fr, -fi
    pq[0, 0:64, 1::2], pq[1, 0:64, 1::2] = -fi, -fr
    pq[0, 64:128, 0::2], pq[1, 64:128, 0::2] = fi, fr
    pq[0, 64:128, 1::2], pq[1, 64:128, 1::2] = fr, -fi
    ang = -2.0 * np.pi * np.outer(n1, n2) / S
    tw = np.stack([np.repeat(np.cos(ang), 2, axis=1), np.repeat(np.sin(ang), 2, axis=1)])
    gt = np.concatenate([pq.reshape(256, 128), tw.reshape(64, 128)]).astype(np.float32)
    tb = lambda a: np.asarray(a, dtype=np.float32).astype(BF)
    rf = np.stack([rf[:, :128], rf[:, 128:]])
    ci = np.stack([ci[0, :, :128], ci[0, :, 128:], ci[1, :, :128], ci[1, :, 128:]])
    return tb(rf), tb(ci), tb(fa), gt


_RF, _CI, _FA, _GT = _consts()


def _nn(a, b):
    return jnp.dot(a, b, preferred_element_type=F32)


def _nt(a, b):
    return lax.dot_general(a, b, (((1,), (1,)), ((), ())), preferred_element_type=F32)


def _tn(a, b):
    return lax.dot_general(a, b, (((0,), (0,)), ((), ())), preferred_element_type=F32)


def _run(g):
    for _ in g:
        pass


def _seq(*gs):
    for g in gs:
        yield from g


def _rr(*gs):
    gs = list(gs)
    while gs:
        nxt = []
        for g in gs:
            try:
                next(g)
                nxt.append(g)
            except StopIteration:
                pass
        gs = nxt
        yield


NRF = (240, 224)
NT = S // 128
XT = (0, 3, 7, 11, 16)
NXC = len(XT) - 1
BM = 512
NB = S // BM
Q = D // 4
NC2 = 3
F1 = 512 * NC2
RC = 32
RP = 16
NKT = FF // 256


def _take(g, n):
    for _ in range(n):
        try:
            next(g)
        except StopIteration:
            return
        yield


def _mix(ga, na, gb, nb):
    k = 0
    for a in range(na):
        next(ga, None)
        while k < (a + 1) * nb // na:
            next(gb, None)
            k += 1
        yield
    _run(ga)
    _run(gb)


def _seven_b(b11, b12, b21, b22):
    return (b11 + b22, b11, b12 - b22, b21 - b11, b22, b11 + b12, b21 + b22)


def _seven_a(a11, a12, a21, a22):
    return (a11 + a22, a21 + a22, a11, a22, a11 + a12, a21 - a11, a12 - a22)


TERMS_A = (((1, 0), (1, 3)), ((1, 2), (1, 3)), ((1, 0),), ((1, 3),),
           ((1, 0), (1, 1)), ((1, 2), (-1, 0)), ((1, 1), (-1, 3)))
TERMS_B = (((1, 0), (1, 3)), ((1, 0),), ((1, 1), (-1, 3)), ((1, 2), (-1, 0)),
           ((1, 3),), ((1, 0), (1, 1)), ((1, 2), (1, 3)))


def _term(terms, get):
    v = get(terms[0][1])
    for sign, q in terms[1:]:
        v = v + get(q) if sign > 0 else v - get(q)
    return v


def _fold8(v):
    parts = [v[r:r + 8] for r in range(0, v.shape[0], 8)]
    while len(parts) > 1:
        parts = [parts[k] + parts[k + 1] if k + 1 < len(parts) else parts[k]
                 for k in range(0, len(parts), 2)]
    return parts[0]


def _combine(m):
    return (m[0] + m[3] - m[4] + m[6], m[2] + m[4], m[1] + m[3], m[0] - m[1] + m[2] + m[5])


def _words(ref):
    return ref.bitcast(U32)


def _bf(w):
    return pltpu.bitcast(w, BF)


def _kernel(x_hbm, wr_hbm, wi_hbm, wg_hbm, wu_hbm, wd_hbm,
            rf_hbm, ci_hbm, fa_hbm, gt_hbm,
            o_hbm,
            x_v, wr_v, wi_v, wg_v, wu_v, wd_v,
            rf_v, ci_v, fa_v, gt_v, gs, xs,
            a0s, ab, zt, ze, zo, ye, yo, ve, vo, wsr, wsi, se, so,
            hb, cn, a2, a1, wg2, wu2, wg1, wu1, wds, hs, ob,
            sem_x, sem_c, sem_o, sem_f):

    def colcp(src, dst, c0, w, sem):
        return pltpu.make_async_copy(src.at[:, pl.ds(c0, w)], dst.at[:, pl.ds(c0, w)], sem)

    xcp = [colcp(x_hbm, x_v, XT[c] * 128, (XT[c + 1] - XT[c]) * 128, sem_x.at[c])
           for c in range(NXC)]
    c_rf = pltpu.make_async_copy(rf_hbm, rf_v, sem_c.at[0])
    c_fa = pltpu.make_async_copy(fa_hbm, fa_v, sem_c.at[1])
    c_ci = pltpu.make_async_copy(ci_hbm, ci_v, sem_c.at[2])
    c_wr = pltpu.make_async_copy(wr_hbm, wr_v, sem_c.at[3])
    c_wi = pltpu.make_async_copy(wi_hbm, wi_v, sem_c.at[4])
    c_gt = pltpu.make_async_copy(gt_hbm, gt_v, sem_c.at[5])
    c_wd = pltpu.make_async_copy(wd_hbm, wd_v, sem_c.at[6])
    wgc = [colcp(wg_hbm, wg_v, a, b - a, sem_c.at[7 + n])
           for n, (a, b) in enumerate(((0, 512), (512, 1024), (1024, FF)))]
    wuc = [colcp(wu_hbm, wu_v, a, b - a, sem_c.at[10 + n])
           for n, (a, b) in enumerate(((0, 512), (512, 1024), (1024, FF)))]
    ocp = [colcp(ob, o_hbm, j * BM, BM, sem_o.at[j]) for j in range(NB - 1)]
    c0 = (NB - 1) * BM
    ocp += [colcp(ob, o_hbm, c0, 256, sem_o.at[NB - 1])]
    ocp += [pltpu.make_async_copy(ob.at[pl.ds(d * H, H), pl.ds(c0 + 256, 256)],
                                  o_hbm.at[pl.ds(d * H, H), pl.ds(c0 + 256, 256)], sem_o.at[NB + d])
            for d in range(2)]

    rf_w, ci_w, fa_w, gs_w = _words(rf_v), _words(ci_v), _words(fa_v), _words(gs)
    ab_w, zt_w = _words(ab), _words(zt)
    ye_w, yo_w, ve_w, vo_w, se_w, so_w = (_words(r) for r in (ye, yo, ve, vo, se, so))
    hb_w, a2_w, a1_w = _words(hb), _words(a2), _words(a1)
    wg2_w, wu2_w, wg1_w, wu1_w = (_words(r) for r in (wg2, wu2, wg1, wu1))
    wds_w, hs_w = _words(wds), _words(hs)

    def ln1(t):
        cols = slice(128 * t, 128 * (t + 1))
        u = t % 2
        acc = None
        for r in range(0, H, RC):
            lo = x_v[r:r + RC, cols].astype(F32)
            hi = x_v[H + r:H + r + RC, cols].astype(F32)
            a0 = lo + hi
            a0s[u, r:r + RC, :] = a0
            a0s[u, H + r:H + r + RC, :] = lo - hi
            part = _fold8(a0)
            acc = part if acc is None else acc + part
        m2 = jnp.sum(acc, axis=0, keepdims=True) * (2.0 / D)
        yield
        acc = None
        for r in range(0, H, RC):
            ca = a0s[u, r:r + RC, :] - m2
            b0 = a0s[u, H + r:H + r + RC, :]
            part = _fold8(ca * ca + b0 * b0)
            acc = part if acc is None else acc + part
        rs = lax.rsqrt(jnp.sum(acc, axis=0, keepdims=True) * (0.5 / D) + EPS)
        yield
        for r in range(0, H, RC):
            ab[t, r:r + RC, :] = ((a0s[u, r:r + RC, :] - m2) * rs).astype(BF)
            ab[t, H + r:H + r + RC, :] = (a0s[u, H + r:H + r + RC, :] * rs).astype(BF)
        yield

    def dfwd(t):
        for e in range(2):
            n = NRF[e]
            lhs = jnp.concatenate([_bf(rf_w[0, e * 128:e * 128 + n // 2, :]),
                                   _bf(rf_w[1, e * 128:e * 128 + n // 2, :])[:, :H - 128]], axis=1)
            res = _nn(lhs, _bf(ab_w[t, e * (H // 2):(e + 1) * (H // 2), :]))
            zt[t, e, 0:n, :] = res.astype(BF)

    def dmove(t):
        for e, dst in enumerate((ze, zo)):
            w = zt_w[t, e].T
            for g in range(2):
                dst[pl.ds(PZ * (2 * t + g), N2), :] = w[N2 * g:N2 * (g + 1)]

    row8 = lax.broadcasted_iota(jnp.int32, (8, 128), 0)

    def wprep(t, src, dst):
        wd_ = pltpu.bitcast(src[0:H, t * 128:(t + 1) * 128], U32)
        ny = src[H:H + 1, t * 128:(t + 1) * 128].astype(F32)
        ny = pltpu.bitcast(jnp.broadcast_to(ny, (8, 128)), U32) >> 16
        ny = jnp.where(row8 == 0, ny, jnp.zeros_like(ny))
        wt = jnp.concatenate([wd_, ny, jnp.zeros((8, 128), U32)], axis=0).T
        for g in range(4):
            dst[pl.ds(PW * (4 * t + g), N1), :] = wt[N1 * g:N1 * (g + 1)]
        yield

    def gather2(src, s0, s1, pitch):
        return _bf(jnp.concatenate([src[pl.ds(s0, N1, stride=pitch), :],
                                    src[pl.ds(s1, N1, stride=pitch), :]], axis=0))

    def stage_a(ps, waits=()):
        rhs = jnp.concatenate([gather2(z, p, p + N1, PZ) for p in ps for z in (ze, zo)], axis=1)
        res = _nn(_bf(fa_w[0]), rhs)
        for c in waits:
            c.wait()
        i = 0
        for p in ps:
            for y in (ye, yo):
                y[pl.ds(2 * PY * p, 128), :] = res[:, i * 128:(i + 1) * 128].astype(BF)
                i += 1
        yield

    def stage_b(k1, waits=()):
        g = (gt_v[0:128, :] * gt_v[256 + k1:257 + k1, :]
             + gt_v[128:256, :] * gt_v[288 + k1:289 + k1, :]).astype(BF)
        gs[k1] = g
        rhs = jnp.concatenate([gather2(y, k1, N1 + k1, PY) for y in (ye_w, yo_w)], axis=1)
        xx = _nn(g, rhs)
        for c in waits:
            c.wait()
        xs[k1, 0] = xx[:, :128]
        xs[k1, 1] = xx[:, 128:]
        yield

    def stage_bi(k1):
        wr = wsr[pl.ds(k1, N2, stride=PW), :]
        wi = wsi[pl.ds(k1, N2, stride=PW), :]
        par = ((wr << 16, wi << 16),
               (wr & jnp.uint32(0xFFFF0000), wi & jnp.uint32(0xFFFF0000)))
        tiles = []
        for e in range(2):
            w_r, w_i = (pltpu.bitcast(w, F32) for w in par[e])
            x_r, x_i = xs[k1, e, 0:N2, :], xs[k1, e, N2:128, :]
            tiles.append(jnp.concatenate([x_r * w_r - x_i * w_i, x_r * w_i + x_i * w_r],
                                         axis=0).astype(BF))
        yy = _nn(_bf(gs_w[k1]).T, jnp.concatenate(tiles, axis=1))
        ve[pl.ds(2 * PY * k1, 128), :] = yy[:, :128].astype(BF)
        vo[pl.ds(2 * PY * k1, 128), :] = yy[:, 128:].astype(BF)
        yield

    def stage_ai(ps, side=None):
        rhs = jnp.concatenate([gather2(v, 2 * p, 2 * p + 1, PY) for p in ps for v in (ve_w, vo_w)],
                              axis=1)
        res = _nn(_bf(fa_w[1]), rhs)
        if side is not None:
            side((pltpu.bitcast(res[0:8, 0:128], U32) | 1) == 0)
        i = 0
        for p in ps:
            for y in (se, so):
                y[pl.ds(2 * PY * p, 128), :] = res[:, i * 128:(i + 1) * 128].astype(BF)
                i += 1
        yield

    def prep_tiles(j, tiles):
        def inv_d(e, src):
            rhs = jnp.concatenate(
                [jnp.concatenate(
                    [_bf(jnp.concatenate([src[pl.ds(ro * N1 + 2 * (4 * j + i) + g, N1, stride=PY), :]
                                          for g in range(2)], axis=0))
                     for ro in range(2)], axis=1) for i in tiles], axis=0)
            lhs = jnp.concatenate([_bf(ci_w[2 * e]), _bf(ci_w[2 * e + 1])], axis=1)
            return _nt(lhs, rhs)
        ep = inv_d(0, se_w)
        op = inv_d(1, so_w)
        for n, i in enumerate(tiles):
            t = 4 * j + i
            cols = slice(128 * n, 128 * (n + 1))
            acc = None
            for r in range(0, H, RC):
                e, o = ep[r:r + RC, cols], op[r:r + RC, cols]
                lo = x_v[r:r + RC, t * 128:(t + 1) * 128].astype(F32) + (e + o)
                hi = x_v[H + r:H + r + RC, t * 128:(t + 1) * 128].astype(F32) + (e - o)
                for r0, v in ((r, lo), (H + r, hi)):
                    hb[j % 2, i, r0:r0 + RC, :] = v.astype(BF)
                    cn[i, r0:r0 + RC, :] = v
                part = _fold8(lo + hi)
                acc = part if acc is None else acc + part
            m = jnp.sum(acc, axis=0, keepdims=True) * (1.0 / D)
            acc = None
            for r in range(0, D, 2 * RC):
                c = cn[i, r:r + 2 * RC, :] - m
                part = _fold8(c * c)
                acc = part if acc is None else acc + part
            rs = lax.rsqrt(jnp.sum(acc, axis=0, keepdims=True) * (1.0 / D) + EPS)
            for r in range(0, D, 2 * RC):
                cn[i, r:r + 2 * RC, :] = (cn[i, r:r + 2 * RC, :] - m) * rs

    def prep_ops():
        blk = lambda mh, kh, ml, kl: cn[2 * mh + ml, Q * (2 * kh + kl):Q * (2 * kh + kl + 1), :]
        zpad = jnp.zeros((128 - Q, 128), F32)

        def put(dst_w, idx, v):
            dst_w[idx] = pltpu.bitcast(jnp.concatenate([v, zpad], axis=0).astype(BF).T, U32)

        def lvl1(i, ml, kl):
            return _term(TERMS_A[i], lambda q: blk(q // 2, q % 2, ml, kl))

        for i in range(7):
            for ml in range(2):
                for kl in range(2):
                    put(a1_w, (i, ml, kl), lvl1(i, ml, kl))
            for k in range(7):
                put(a2_w, (7 * i + k,), _term(TERMS_A[k], lambda q: lvl1(i, q // 2, q % 2)))

    def wblk(w_v, kq, f0, r, tie=None):
        v = w_v[Q * kq + r:Q * kq + r + RP, f0:f0 + 128].astype(F32)
        if tie is not None:
            v = jnp.where(jnp.concatenate([tie] * (RP // 8), axis=0), 0.0, v)
        return v

    def build2(w_v, w2, c, i, tie=None):
        for r in range(0, Q, RP):
            ri = [[_term(TERMS_B[i], lambda q: wblk(w_v, 2 * (q // 2) + kl,
                                                    512 * c + 128 * (2 * (q % 2) + fl), r, tie))
                   for fl in range(2)] for kl in range(2)]
            ops = _seven_b(ri[0][0], ri[0][1], ri[1][0], ri[1][1])
            for k in range(7):
                w2[c, 7 * i + k, r:r + RP, :] = ops[k].astype(BF)

    def store_hs(kt, pair, q11, q21, q12, q22):
        ops = _seven_b(q11, q21, q12, q22)
        for i in range(7):
            hs[i, kt, pair * 128:(pair + 1) * 128, :] = ops[i].astype(BF)

    def gate2(j, c):
        res = []
        for w_v, w2, w2_w in ((wg_v, wg2, wg2_w), (wu_v, wu2, wu2_w)):
            mm = []
            for i in range(7):
                if j == 0 and c > 0:
                    build2(w_v, w2, c, i)
                ops = [_bf(w2_w[c, 7 * i + k]) for k in range(7)]
                mm.append(_combine([_nn(_bf(a2_w[7 * i + k])[:, :Q], ops[k]) for k in range(7)]))
                yield
            res.append([_combine([mm[i][t] for i in range(7)]) for t in range(4)])
        q = [[res[0][t][o] * res[1][t][o] for o in range(4)] for t in range(4)]
        tile = lambda mt, ft: q[(mt % 2) * 2 + ft % 2][(mt // 2) * 2 + ft // 2]
        for fl in range(2):
            for ml in range(2):
                store_hs(2 * c + fl, ml, tile(ml, fl), tile(2 + ml, fl), tile(ml, 2 + fl), tile(2 + ml, 2 + fl))
        yield

    def gate1(j):
        res = []
        for w_v, w1, w1_w in ((wg_v, wg1, wg1_w), (wu_v, wu1, wu1_w)):
            if j == 0:
                for kl in range(2):
                    for r in range(0, Q, RP):
                        ops = _seven_b(wblk(w_v, kl, F1, r), wblk(w_v, kl, F1 + 128, r),
                                       wblk(w_v, 2 + kl, F1, r), wblk(w_v, 2 + kl, F1 + 128, r))
                        for i in range(7):
                            w1[i, kl, r:r + RP, :] = ops[i].astype(BF)
            ops = [[_bf(w1_w[i, kl]) for i in range(7)] for kl in range(2)]
            m = []
            for i in range(7):
                part = [_nn(jnp.concatenate([_bf(a1_w[i, ml, kl])[:, :Q] for ml in range(2)], axis=0),
                            ops[kl][i]) for kl in range(2)]
                m.append(part[0] + part[1])
            res.append(_combine(m))
        q11, q12, q21, q22 = [g_ * u_ for g_, u_ in zip(*res)]
        for ml in range(2):
            sl = slice(128 * ml, 128 * (ml + 1))
            store_hs(NKT - 1, ml, q11[sl], q21[sl], q12[sl], q22[sl])
        yield

    def wd_cols(kt, fh):
        if kt < 2 * NC2:
            return 512 * (kt // 2) + 128 * (kt % 2) + 256 * fh
        return F1 + 128 * fh

    def down(j):
        if j == 0:
            for kt in range(NKT):
                for r in range(0, H, 2 * RP):
                    quad = lambda d, fh: wd_v[H * d + r:H * d + r + 2 * RP,
                                              wd_cols(kt, fh):wd_cols(kt, fh) + 128].astype(F32)
                    ops = _seven_a(quad(0, 0), quad(0, 1), quad(1, 0), quad(1, 1))
                    for i in range(7):
                        wds[i, kt, r:r + 2 * RP, :] = ops[i].astype(BF)
        ops = [[_bf(wds_w[i, kt]) for i in range(7)] for kt in range(NKT)]
        m = [None] * 7
        for i in (0, 1, 3, 4, 6, 2, 5):
            lhs = jnp.concatenate([ops[kt][i] for kt in range(NKT)], axis=1)
            rhs = jnp.concatenate([_bf(hs_w[i, kt]) for kt in range(NKT)], axis=1)
            m[i] = _nt(lhs, rhs)
            yield
        o11, o12, o21, o22 = _combine(m)
        for mh, halves in enumerate(((o11, o21), (o12, o22))):
            for d, o in enumerate(halves):
                for ml in range(2):
                    i = 2 * mh + ml
                    t = 4 * j + i
                    hh_ = _bf(hb_w[j % 2, i, d * (H // 2):(d + 1) * (H // 2), :]).astype(F32)
                    ob[d * H:(d + 1) * H, t * 128:(t + 1) * 128] = (
                        hh_ + o[:, 128 * ml:128 * (ml + 1)]).astype(BF)
                if j == NB - 1 and mh == 1:
                    ocp[NB + d].start()
            if j == NB - 1 and mh == 0:
                ocp[j].start()
        if j < NB - 1:
            ocp[j].start()

    for c in (xcp[0], c_rf, *xcp[1:], c_fa, c_wr, c_gt, c_wi, c_ci,
              wgc[0], wuc[0], wgc[1], wuc[1], wgc[2], wuc[2], c_wd):
        c.start()
        pl.semaphore_signal(sem_f, 1)
        pl.semaphore_wait(sem_f, 1)
    for e in range(2):
        zt[:, e, NRF[e]:256, :] = jnp.zeros((NT, 256 - NRF[e], 128), BF)
    xcp[0].wait()
    seed = x_v[0:8, 0:128]
    for buf in (ab, zt, gs, hb, a2, a1, wg2, wu2, wg1, wu1, wds, hs):
        buf[(0,) * (len(buf.shape) - 2) + (slice(0, 8), slice(None))] = seed
    for buf in (xs, cn, a0s):
        buf[(0,) * (len(buf.shape) - 2) + (slice(0, 1), slice(None))] = seed[0:1].astype(F32)
    for t in range(XT[0], XT[1]):
        _run(ln1(t))
    c_rf.wait()
    DEF = 1
    for c in range(NXC):
        for t in range(XT[c], XT[c + 1]):
            if c > 0:
                _run(ln1(t))
            dfwd(t)
            if t < XT[c + 1] - DEF or c + 1 == NXC:
                dmove(t)
        if c + 1 < NXC:
            xcp[c + 1].wait()
            for t in range(XT[c + 1] - DEF, XT[c + 1]):
                dmove(t)
    NG = N1 // 2
    c_fa.wait()
    _run(_seq(*[stage_a([2 * g, 2 * g + 1]) for g in range(NG // 2 - 1)]))
    _run(stage_a([NG - 2, NG - 1], waits=(c_wr,)))
    _run(_mix(_seq(*[stage_a([2 * g, 2 * g + 1]) for g in range(NG // 2, NG)]), NG // 2,
              _seq(*[wprep(t, wr_v, wsr) for t in range(NT)]), NT))
    c_gt.wait()
    _run(_seq(*[stage_b(k1) for k1 in range(N1 // 2 - 1)]))
    _run(stage_b(N1 // 2 - 1, waits=(c_wi,)))
    _run(_mix(_seq(*[stage_b(k1) for k1 in range(N1 // 2, N1)]), N1 // 2,
              _seq(*[wprep(t, wi_v, wsi) for t in range(NT)]), NT))
    for k1 in range(N1):
        _run(stage_bi(k1))
    c_ci.wait()
    for c in (*wgc[:2], *wuc[:2]):
        c.wait()
    for g in range(NG):
        side = None
        if g < 14:
            side = lambda tie, g=g: build2(*((wg_v, wg2), (wu_v, wu2))[g // 7], 0, g % 7, tie)
        _run(stage_ai([2 * g, 2 * g + 1], side))
    for i in range(4):
        prep_tiles(0, (i,))
    prep_ops()
    for j in range(NB):
        for c in range(NC2 + 1):
            for n, _ in enumerate(gate2(j, c) if c < NC2 else gate1(j)):
                if (j, c, n) == (0, 1, 9):
                    wgc[2].wait()
                    wuc[2].wait()
                    c_wd.wait()
        for n, _ in enumerate(down(j)):
            if j + 1 < NB and n < 4:
                prep_tiles(j + 1, (n,))
            if j + 1 < NB and n == 4:
                prep_ops()
    for c in ocp:
        c.wait()


def _skip(n):
    for _ in range(n):
        yield


@jax.jit
def pallas_sequential_preLN__spectral_gfnet__glu_gated_bilinear__prompt_kernel(
    A_x, A_w_r, A_w_i, B_x, B_w_gate, B_w_up, B_w_down,
):
    del B_x
    xT = jnp.transpose(A_x.reshape(S, D))
    any_spec = pl.BlockSpec(memory_space=pl.ANY)
    vm = pltpu.VMEM
    dma = pltpu.SemaphoreType.DMA
    slab = vm((2 * PY * N1, 128), BF)
    oT = pl.pallas_call(
        _kernel,
        out_shape=jax.ShapeDtypeStruct((D, S), BF),
        in_specs=[any_spec] * 10,
        out_specs=any_spec,
        scratch_shapes=[
            vm((D, S), BF), vm((H + 1, S), BF), vm((H + 1, S), BF),
            vm((D, FF), BF), vm((D, FF), BF), vm((D, FF), BF),
            vm(_RF.shape, BF), vm(_CI.shape, BF), vm(_FA.shape, BF), vm(_GT.shape, F32),
            vm((N1, 128, 128), BF), vm((N1, 2, 128, 128), F32),
            vm((2, D, 128), F32), vm((NT, D, 128), BF), vm((NT, 2, 256, 128), BF),
            vm((N1 * PZ, 128), U32), vm((N1 * PZ, 128), U32),
            slab, slab, slab, slab,
            vm((N2 * PW, 128), U32), vm((N2 * PW, 128), U32),
            slab, slab,
            vm((2, 4, D, 128), BF), vm((4, D, 128), F32),
            vm((49, 128, 128), BF), vm((7, 2, 2, 128, 128), BF),
            vm((NC2, 49, Q, 128), BF), vm((NC2, 49, Q, 128), BF),
            vm((7, 2, Q, 128), BF), vm((7, 2, Q, 128), BF),
            vm((7, NKT, H, 128), BF), vm((7, NKT, 256, 128), BF), vm((D, S), BF),
            dma((NXC,)), dma((13,)), dma((NB + 2,)), pltpu.SemaphoreType.REGULAR,
        ],
        compiler_params=pltpu.CompilerParams(vmem_limit_bytes=100 * 1024 * 1024),
        name="gfnet_glu",
    )(xT, A_w_r.T, A_w_i.T, B_w_gate, B_w_up, B_w_down.T, _RF, _CI, _FA, _GT)
    return jnp.transpose(oT).reshape(1, S, D)
```

```python
import numpy as np
import jax
import jax.numpy as jnp
from jax import lax
from jax.experimental import pallas as pl
from jax.experimental.pallas import tpu as pltpu

S, D, FF = 2048, 448, 1792
H = D // 2
N1, N2 = 32, 64
PZ = N2 + 1
PW = N1 + 1
PY = N2 + 4
BF = jnp.bfloat16
F32 = jnp.float32
U32 = jnp.uint32
EPS = 1e-5


def _consts():
    d = np.arange(H)
    rf = np.zeros((512, 256))
    for m in range(H // 2 + 1):
        ang = -2.0 * np.pi * ((2 * m * d) % D) / D
        rf[2 * m, :H] = np.cos(ang)
        rf[2 * m + 1, :H] = np.sin(ang)
    for m in range(H // 2):
        ang = -2.0 * np.pi * (((2 * m + 1) * d) % D) / D
        rf[256 + 2 * m, :H] = np.cos(ang)
        rf[256 + 2 * m + 1, :H] = np.sin(ang)
    ci = np.zeros((2, H, 256))
    for m in range(H // 2 + 1):
        k = 2 * m
        c = 1.0 if (k == 0 or k == H) else 2.0
        ang = 2.0 * np.pi * ((k * d) % D) / D
        ci[0, :, m] = c * np.cos(ang) / (S * D)
        if k != 0 and k != H:
            ci[0, :, 128 + m] = -c * np.sin(ang) / (S * D)
    for m in range(H // 2):
        k = 2 * m + 1
        ang = 2.0 * np.pi * ((k * d) % D) / D
        ci[1, :, m] = 2.0 * np.cos(ang) / (S * D)
        ci[1, :, 128 + m] = -2.0 * np.sin(ang) / (S * D)
    n1 = np.arange(N1)
    n2 = np.arange(N2)
    ang = -2.0 * np.pi * ((np.outer(n1, n1)) % N1) / N1
    fr, fi = np.cos(ang), np.sin(ang)
    fa = np.zeros((2, 128, 128))
    for mu in range(2):
        o = 64 * mu
        fa[0, o + 0:o + 64:2, o + 0:o + 64:2] = fr
        fa[0, o + 0:o + 64:2, o + 1:o + 64:2] = -fi
        fa[0, o + 1:o + 64:2, o + 0:o + 64:2] = fi
        fa[0, o + 1:o + 64:2, o + 1:o + 64:2] = fr
        fa[1, mu:64:2, o + 0:o + 64:2] = fr
        fa[1, mu:64:2, o + 1:o + 64:2] = fi
        fa[1, 64 + mu:128:2, o + 0:o + 64:2] = -fi
        fa[1, 64 + mu:128:2, o + 1:o + 64:2] = fr
    ang = -2.0 * np.pi * (np.outer(n2, n2) % N2) / N2
    fr, fi = np.cos(ang), np.sin(ang)
    pq = np.zeros((2, 128, 128))
    pq[0, 0:64, 0::2], pq[1, 0:64, 0::2] = fr, -fi
    pq[0, 0:64, 1::2], pq[1, 0:64, 1::2] = -fi, -fr
    pq[0, 64:128, 0::2], pq[1, 64:128, 0::2] = fi, fr
    pq[0, 64:128, 1::2], pq[1, 64:128, 1::2] = fr, -fi
    ang = -2.0 * np.pi * np.outer(n1, n2) / S
    tw = np.stack([np.repeat(np.cos(ang), 2, axis=1), np.repeat(np.sin(ang), 2, axis=1)])
    gt = np.concatenate([pq.reshape(256, 128), tw.reshape(64, 128)]).astype(np.float32)
    tb = lambda a: np.asarray(a, dtype=np.float32).astype(BF)
    rf = np.stack([rf[:, :128], rf[:, 128:]])
    ci = np.stack([ci[0, :, :128], ci[0, :, 128:], ci[1, :, :128], ci[1, :, 128:]])
    return tb(rf), tb(ci), tb(fa), gt


_RF, _CI, _FA, _GT = _consts()


def _nn(a, b):
    return jnp.dot(a, b, preferred_element_type=F32)


def _nt(a, b):
    return lax.dot_general(a, b, (((1,), (1,)), ((), ())), preferred_element_type=F32)


def _run(g):
    for _ in g:
        pass


def _seq(*gs):
    for g in gs:
        yield from g


NRF = (240, 224)
NT = S // 128
XT = (0, 3, 7, 11, 16)
NXC = len(XT) - 1
BM = 512
NB = S // BM
Q = D // 4
NC2 = 3
F1 = 512 * NC2
RC = 32
RP = 16
NKT = FF // 256


def _mix(ga, na, gb, nb):
    k = 0
    for a in range(na):
        next(ga, None)
        while k < (a + 1) * nb // na:
            next(gb, None)
            k += 1
        yield
    _run(ga)
    _run(gb)


def _seven_b(b11, b12, b21, b22):
    return (b11 + b22, b11, b12 - b22, b21 - b11, b22, b11 + b12, b21 + b22)


def _seven_a(a11, a12, a21, a22):
    return (a11 + a22, a21 + a22, a11, a22, a11 + a12, a21 - a11, a12 - a22)


TERMS_A = (((1, 0), (1, 3)), ((1, 2), (1, 3)), ((1, 0),), ((1, 3),),
           ((1, 0), (1, 1)), ((1, 2), (-1, 0)), ((1, 1), (-1, 3)))
TERMS_B = (((1, 0), (1, 3)), ((1, 0),), ((1, 1), (-1, 3)), ((1, 2), (-1, 0)),
           ((1, 3),), ((1, 0), (1, 1)), ((1, 2), (1, 3)))


def _term(terms, get):
    v = get(terms[0][1])
    for sign, q in terms[1:]:
        v = v + get(q) if sign > 0 else v - get(q)
    return v


def _fold8(v):
    parts = [v[r:r + 8] for r in range(0, v.shape[0], 8)]
    while len(parts) > 1:
        parts = [parts[k] + parts[k + 1] if k + 1 < len(parts) else parts[k]
                 for k in range(0, len(parts), 2)]
    return parts[0]


def _combine(m):
    return (m[0] + m[3] - m[4] + m[6], m[2] + m[4], m[1] + m[3], m[0] - m[1] + m[2] + m[5])


def _words(ref):
    return ref.bitcast(U32)


def _bf(w):
    return pltpu.bitcast(w, BF)


def _kernel(x_hbm, wr_hbm, wi_hbm, wg_hbm, wu_hbm, wd_hbm,
            rf_hbm, ci_hbm, fa_hbm, gt_hbm,
            o_hbm,
            x_v, wr_v, wi_v, wg_v, wu_v, wd_v,
            rf_v, ci_v, fa_v, gt_v, gs, xs,
            a0s, ab, zt, ze, zo, ye, yo, ve, vo, wsr, wsi, se, so,
            hb, cn, a2, a1, wg2, wu2, wg1, wu1, wds, hs, ob,
            sem_x, sem_c, sem_o, sem_f):

    def colcp(src, dst, c0, w, sem):
        return pltpu.make_async_copy(src.at[:, pl.ds(c0, w)], dst.at[:, pl.ds(c0, w)], sem)

    xcp = [colcp(x_hbm, x_v, XT[c] * 128, (XT[c + 1] - XT[c]) * 128, sem_x.at[c])
           for c in range(NXC)]
    c_rf = pltpu.make_async_copy(rf_hbm, rf_v, sem_c.at[0])
    c_fa = pltpu.make_async_copy(fa_hbm, fa_v, sem_c.at[1])
    c_ci = pltpu.make_async_copy(ci_hbm, ci_v, sem_c.at[2])
    c_wr = pltpu.make_async_copy(wr_hbm, wr_v, sem_c.at[3])
    c_wi = pltpu.make_async_copy(wi_hbm, wi_v, sem_c.at[4])
    c_gt = pltpu.make_async_copy(gt_hbm, gt_v, sem_c.at[5])
    c_wd = pltpu.make_async_copy(wd_hbm, wd_v, sem_c.at[6])
    wgc = [colcp(wg_hbm, wg_v, a, b - a, sem_c.at[7 + n])
           for n, (a, b) in enumerate(((0, 512), (512, 1024), (1024, FF)))]
    wuc = [colcp(wu_hbm, wu_v, a, b - a, sem_c.at[10 + n])
           for n, (a, b) in enumerate(((0, 512), (512, 1024), (1024, FF)))]
    ocp = [colcp(ob, o_hbm, j * BM, BM, sem_o.at[j]) for j in range(NB - 1)]
    c0 = (NB - 1) * BM
    ocp += [colcp(ob, o_hbm, c0, 256, sem_o.at[NB - 1])]
    ocp += [pltpu.make_async_copy(ob.at[pl.ds(d * H, H), pl.ds(c0 + 256, 256)],
                                  o_hbm.at[pl.ds(d * H, H), pl.ds(c0 + 256, 256)], sem_o.at[NB + d])
            for d in range(2)]

    rf_w, ci_w, fa_w, gs_w = _words(rf_v), _words(ci_v), _words(fa_v), _words(gs)
    ab_w, zt_w = _words(ab), _words(zt)
    ye_w, yo_w, ve_w, vo_w, se_w, so_w = (_words(r) for r in (ye, yo, ve, vo, se, so))
    hb_w, a2_w, a1_w = _words(hb), _words(a2), _words(a1)
    wg2_w, wu2_w, wg1_w, wu1_w = (_words(r) for r in (wg2, wu2, wg1, wu1))
    wds_w, hs_w = _words(wds), _words(hs)

    def ln1(t):
        cols = slice(128 * t, 128 * (t + 1))
        u = t % 2
        acc = None
        for r in range(0, H, RC):
            lo = x_v[r:r + RC, cols].astype(F32)
            hi = x_v[H + r:H + r + RC, cols].astype(F32)
            a0 = lo + hi
            a0s[u, r:r + RC, :] = a0
            a0s[u, H + r:H + r + RC, :] = lo - hi
            part = _fold8(a0)
            acc = part if acc is None else acc + part
        m2 = jnp.sum(acc, axis=0, keepdims=True) * (2.0 / D)
        yield
        acc = None
        for r in range(0, H, RC):
            ca = a0s[u, r:r + RC, :] - m2
            b0 = a0s[u, H + r:H + r + RC, :]
            part = _fold8(ca * ca + b0 * b0)
            acc = part if acc is None else acc + part
        rs = lax.rsqrt(jnp.sum(acc, axis=0, keepdims=True) * (0.5 / D) + EPS)
        yield
        for r in range(0, H, RC):
            ab[t, r:r + RC, :] = ((a0s[u, r:r + RC, :] - m2) * rs).astype(BF)
            ab[t, H + r:H + r + RC, :] = (a0s[u, H + r:H + r + RC, :] * rs).astype(BF)
        yield

    def dfwd(t):
        for e in range(2):
            n = NRF[e]
            lhs = jnp.concatenate([_bf(rf_w[0, e * 128:e * 128 + n // 2, :]),
                                   _bf(rf_w[1, e * 128:e * 128 + n // 2, :])[:, :H - 128]], axis=1)
            res = _nn(lhs, _bf(ab_w[t, e * (H // 2):(e + 1) * (H // 2), :]))
            zt[t, e, 0:n, :] = res.astype(BF)

    def dmove(t):
        for e, dst in enumerate((ze, zo)):
            w = zt_w[t, e].T
            for g in range(2):
                dst[pl.ds(PZ * (2 * t + g), N2), :] = w[N2 * g:N2 * (g + 1)]

    row8 = lax.broadcasted_iota(jnp.int32, (8, 128), 0)

    def wprep(t, src, dst):
        wd_ = pltpu.bitcast(src[0:H, t * 128:(t + 1) * 128], U32)
        ny = src[H:H + 1, t * 128:(t + 1) * 128].astype(F32)
        ny = pltpu.bitcast(jnp.broadcast_to(ny, (8, 128)), U32) >> 16
        ny = jnp.where(row8 == 0, ny, jnp.zeros_like(ny))
        wt = jnp.concatenate([wd_, ny, jnp.zeros((8, 128), U32)], axis=0).T
        for g in range(4):
            dst[pl.ds(PW * (4 * t + g), N1), :] = wt[N1 * g:N1 * (g + 1)]
        yield

    def gather2(src, s0, s1, pitch):
        return _bf(jnp.concatenate([src[pl.ds(s0, N1, stride=pitch), :],
                                    src[pl.ds(s1, N1, stride=pitch), :]], axis=0))

    def stage_a(ps, waits=()):
        rhs = jnp.concatenate([gather2(z, p, p + N1, PZ) for p in ps for z in (ze, zo)], axis=1)
        res = _nn(_bf(fa_w[0]), rhs)
        for c in waits:
            c.wait()
        i = 0
        for p in ps:
            for y in (ye, yo):
                y[pl.ds(2 * PY * p, 128), :] = res[:, i * 128:(i + 1) * 128].astype(BF)
                i += 1
        yield

    def stage_b(k1, waits=()):
        g = (gt_v[0:128, :] * gt_v[256 + k1:257 + k1, :]
             + gt_v[128:256, :] * gt_v[288 + k1:289 + k1, :]).astype(BF)
        gs[k1] = g
        rhs = jnp.concatenate([gather2(y, k1, N1 + k1, PY) for y in (ye_w, yo_w)], axis=1)
        xx = _nn(g, rhs)
        for c in waits:
            c.wait()
        xs[k1, 0] = xx[:, :128]
        xs[k1, 1] = xx[:, 128:]
        yield

    def stage_bi(k1):
        wr = wsr[pl.ds(k1, N2, stride=PW), :]
        wi = wsi[pl.ds(k1, N2, stride=PW), :]
        par = ((wr << 16, wi << 16),
               (wr & jnp.uint32(0xFFFF0000), wi & jnp.uint32(0xFFFF0000)))
        tiles = []
        for e in range(2):
            w_r, w_i = (pltpu.bitcast(w, F32) for w in par[e])
            x_r, x_i = xs[k1, e, 0:N2, :], xs[k1, e, N2:128, :]
            tiles.append(jnp.concatenate([x_r * w_r - x_i * w_i, x_r * w_i + x_i * w_r],
                                         axis=0).astype(BF))
        yy = _nn(_bf(gs_w[k1]).T, jnp.concatenate(tiles, axis=1))
        ve[pl.ds(2 * PY * k1, 128), :] = yy[:, :128].astype(BF)
        vo[pl.ds(2 * PY * k1, 128), :] = yy[:, 128:].astype(BF)
        yield

    def stage_ai(ps, side=None):
        rhs = jnp.concatenate([gather2(v, 2 * p, 2 * p + 1, PY) for p in ps for v in (ve_w, vo_w)],
                              axis=1)
        res = _nn(_bf(fa_w[1]), rhs)
        if side is not None:
            side((pltpu.bitcast(res[0:8, 0:128], U32) | 1) == 0)
        i = 0
        for p in ps:
            for y in (se, so):
                y[pl.ds(2 * PY * p, 128), :] = res[:, i * 128:(i + 1) * 128].astype(BF)
                i += 1
        yield

    def prep_tiles(j, tiles):
        def inv_d(e, src):
            rhs = jnp.concatenate(
                [jnp.concatenate(
                    [_bf(jnp.concatenate([src[pl.ds(ro * N1 + 2 * (4 * j + i) + g, N1, stride=PY), :]
                                          for g in range(2)], axis=0))
                     for ro in range(2)], axis=1) for i in tiles], axis=0)
            lhs = jnp.concatenate([_bf(ci_w[2 * e]), _bf(ci_w[2 * e + 1])], axis=1)
            return _nt(lhs, rhs)
        ep = inv_d(0, se_w)
        op = inv_d(1, so_w)
        for n, i in enumerate(tiles):
            t = 4 * j + i
            cols = slice(128 * n, 128 * (n + 1))
            acc = None
            for r in range(0, H, RC):
                e, o = ep[r:r + RC, cols], op[r:r + RC, cols]
                lo = x_v[r:r + RC, t * 128:(t + 1) * 128].astype(F32) + (e + o)
                hi = x_v[H + r:H + r + RC, t * 128:(t + 1) * 128].astype(F32) + (e - o)
                for r0, v in ((r, lo), (H + r, hi)):
                    hb[j % 2, i, r0:r0 + RC, :] = v.astype(BF)
                    cn[i, r0:r0 + RC, :] = v
                part = _fold8(lo + hi)
                acc = part if acc is None else acc + part
            m = jnp.sum(acc, axis=0, keepdims=True) * (1.0 / D)
            acc = None
            for r in range(0, D, 2 * RC):
                c = cn[i, r:r + 2 * RC, :] - m
                part = _fold8(c * c)
                acc = part if acc is None else acc + part
            rs = lax.rsqrt(jnp.sum(acc, axis=0, keepdims=True) * (1.0 / D) + EPS)
            for r in range(0, D, 2 * RC):
                cn[i, r:r + 2 * RC, :] = (cn[i, r:r + 2 * RC, :] - m) * rs

    def prep_ops():
        blk = lambda mh, kh, ml, kl: cn[2 * mh + ml, Q * (2 * kh + kl):Q * (2 * kh + kl + 1), :]
        zpad = jnp.zeros((128 - Q, 128), F32)

        def put(dst_w, idx, v):
            dst_w[idx] = pltpu.bitcast(jnp.concatenate([v, zpad], axis=0).astype(BF).T, U32)

        def lvl1(i, ml, kl):
            return _term(TERMS_A[i], lambda q: blk(q // 2, q % 2, ml, kl))

        for i in range(7):
            for ml in range(2):
                for kl in range(2):
                    put(a1_w, (i, ml, kl), lvl1(i, ml, kl))
            for k in range(7):
                put(a2_w, (7 * i + k,), _term(TERMS_A[k], lambda q: lvl1(i, q // 2, q % 2)))

    def wblk(w_v, kq, f0, r, tie=None):
        v = w_v[Q * kq + r:Q * kq + r + RP, f0:f0 + 128].astype(F32)
        if tie is not None:
            v = jnp.where(jnp.concatenate([tie] * (RP // 8), axis=0), 0.0, v)
        return v

    def build2(w_v, w2, c, i, tie=None):
        for r in range(0, Q, RP):
            ri = [[_term(TERMS_B[i], lambda q: wblk(w_v, 2 * (q // 2) + kl,
                                                    512 * c + 128 * (2 * (q % 2) + fl), r, tie))
                   for fl in range(2)] for kl in range(2)]
            ops = _seven_b(ri[0][0], ri[0][1], ri[1][0], ri[1][1])
            for k in range(7):
                w2[c, 7 * i + k, r:r + RP, :] = ops[k].astype(BF)

    def store_hs(kt, pair, q11, q21, q12, q22):
        ops = _seven_b(q11, q21, q12, q22)
        for i in range(7):
            hs[i, kt, pair * 128:(pair + 1) * 128, :] = ops[i].astype(BF)

    def gate2(j, c):
        res = []
        for w_v, w2, w2_w in ((wg_v, wg2, wg2_w), (wu_v, wu2, wu2_w)):
            mm = []
            for i in range(7):
                if j == 0 and c > 0:
                    build2(w_v, w2, c, i)
                ops = [_bf(w2_w[c, 7 * i + k]) for k in range(7)]
                mm.append(_combine([_nn(_bf(a2_w[7 * i + k])[:, :Q], ops[k]) for k in range(7)]))
                yield
            res.append([_combine([mm[i][t] for i in range(7)]) for t in range(4)])
        q = [[res[0][t][o] * res[1][t][o] for o in range(4)] for t in range(4)]
        tile = lambda mt, ft: q[(mt % 2) * 2 + ft % 2][(mt // 2) * 2 + ft // 2]
        for fl in range(2):
            for ml in range(2):
                store_hs(2 * c + fl, ml, tile(ml, fl), tile(2 + ml, fl), tile(ml, 2 + fl), tile(2 + ml, 2 + fl))
        yield

    def gate1(j):
        res = []
        for w_v, w1, w1_w in ((wg_v, wg1, wg1_w), (wu_v, wu1, wu1_w)):
            if j == 0:
                for kl in range(2):
                    for r in range(0, Q, RP):
                        ops = _seven_b(wblk(w_v, kl, F1, r), wblk(w_v, kl, F1 + 128, r),
                                       wblk(w_v, 2 + kl, F1, r), wblk(w_v, 2 + kl, F1 + 128, r))
                        for i in range(7):
                            w1[i, kl, r:r + RP, :] = ops[i].astype(BF)
            ops = [[_bf(w1_w[i, kl]) for i in range(7)] for kl in range(2)]
            m = []
            for i in range(7):
                part = [_nn(jnp.concatenate([_bf(a1_w[i, ml, kl])[:, :Q] for ml in range(2)], axis=0),
                            ops[kl][i]) for kl in range(2)]
                m.append(part[0] + part[1])
            res.append(_combine(m))
        q11, q12, q21, q22 = [g_ * u_ for g_, u_ in zip(*res)]
        for ml in range(2):
            sl = slice(128 * ml, 128 * (ml + 1))
            store_hs(NKT - 1, ml, q11[sl], q21[sl], q12[sl], q22[sl])
        yield

    def wd_cols(kt, fh):
        if kt < 2 * NC2:
            return 512 * (kt // 2) + 128 * (kt % 2) + 256 * fh
        return F1 + 128 * fh

    def down(j):
        if j == 0:
            for kt in range(NKT):
                for r in range(0, H, 2 * RP):
                    quad = lambda d, fh: wd_v[H * d + r:H * d + r + 2 * RP,
                                              wd_cols(kt, fh):wd_cols(kt, fh) + 128].astype(F32)
                    ops = _seven_a(quad(0, 0), quad(0, 1), quad(1, 0), quad(1, 1))
                    for i in range(7):
                        wds[i, kt, r:r + 2 * RP, :] = ops[i].astype(BF)
        ops = [[_bf(wds_w[i, kt]) for i in range(7)] for kt in range(NKT)]
        m = [None] * 7
        for i in (0, 1, 3, 4, 6, 2, 5):
            lhs = jnp.concatenate([ops[kt][i] for kt in range(NKT)], axis=1)
            rhs = jnp.concatenate([_bf(hs_w[i, kt]) for kt in range(NKT)], axis=1)
            m[i] = _nt(lhs, rhs)
            yield
        o11, o12, o21, o22 = _combine(m)
        for mh, halves in enumerate(((o11, o21), (o12, o22))):
            for d, o in enumerate(halves):
                for ml in range(2):
                    i = 2 * mh + ml
                    t = 4 * j + i
                    hh_ = _bf(hb_w[j % 2, i, d * (H // 2):(d + 1) * (H // 2), :]).astype(F32)
                    ob[d * H:(d + 1) * H, t * 128:(t + 1) * 128] = (
                        hh_ + o[:, 128 * ml:128 * (ml + 1)]).astype(BF)
                if j == NB - 1 and mh == 1:
                    ocp[NB + d].start()
            if j == NB - 1 and mh == 0:
                ocp[j].start()
        if j < NB - 1:
            ocp[j].start()

    for c in (xcp[0], c_rf, *xcp[1:], c_fa, c_wr, c_gt, c_wi, c_ci,
              wgc[0], wuc[0], wgc[1], wuc[1], wgc[2], wuc[2], c_wd):
        c.start()
        pl.semaphore_signal(sem_f, 1)
        pl.semaphore_wait(sem_f, 1)
    for e in range(2):
        zt[:, e, NRF[e]:256, :] = jnp.zeros((NT, 256 - NRF[e], 128), BF)
    xcp[0].wait()
    seed = x_v[0:8, 0:128]
    for buf in (ab, zt, gs, hb, a2, a1, wg2, wu2, wg1, wu1, wds, hs):
        buf[(0,) * (len(buf.shape) - 2) + (slice(0, 8), slice(None))] = seed
    for buf in (xs, cn, a0s):
        buf[(0,) * (len(buf.shape) - 2) + (slice(0, 1), slice(None))] = seed[0:1].astype(F32)
    for t in range(XT[0], XT[1]):
        _run(ln1(t))
    c_rf.wait()
    for c in range(NXC):
        for t in range(XT[c], XT[c + 1]):
            if c > 0:
                _run(ln1(t))
            dfwd(t)
            if t < XT[c + 1] - 1 or c + 1 == NXC:
                dmove(t)
        if c + 1 < NXC:
            xcp[c + 1].wait()
            dmove(XT[c + 1] - 1)
    NG = N1 // 2
    c_fa.wait()
    _run(_seq(*[stage_a([2 * g, 2 * g + 1]) for g in range(NG // 2 - 1)]))
    _run(stage_a([NG - 2, NG - 1], waits=(c_wr,)))
    _run(_mix(_seq(*[stage_a([2 * g, 2 * g + 1]) for g in range(NG // 2, NG)]), NG // 2,
              _seq(*[wprep(t, wr_v, wsr) for t in range(NT)]), NT))
    c_gt.wait()
    _run(_seq(*[stage_b(k1) for k1 in range(N1 // 2 - 1)]))
    _run(stage_b(N1 // 2 - 1, waits=(c_wi,)))
    _run(_mix(_seq(*[stage_b(k1) for k1 in range(N1 // 2, N1)]), N1 // 2,
              _seq(*[wprep(t, wi_v, wsi) for t in range(NT)]), NT))
    for k1 in range(N1):
        _run(stage_bi(k1))
    c_ci.wait()
    for c in (*wgc[:2], *wuc[:2]):
        c.wait()
    for g in range(NG):
        side = None
        if g < 14:
            side = lambda tie, g=g: build2(*((wg_v, wg2), (wu_v, wu2))[g // 7], 0, g % 7, tie)
        _run(stage_ai([2 * g, 2 * g + 1], side))
    for i in range(4):
        prep_tiles(0, (i,))
    prep_ops()
    for j in range(NB):
        for c in range(NC2 + 1):
            for n, _ in enumerate(gate2(j, c) if c < NC2 else gate1(j)):
                if (j, c, n) == (0, 1, 13):
                    wgc[2].wait()
                    wuc[2].wait()
                    c_wd.wait()
        for n, _ in enumerate(down(j)):
            if j + 1 < NB and n < 4:
                prep_tiles(j + 1, (n,))
            if j + 1 < NB and n == 4:
                prep_ops()
    for c in ocp:
        c.wait()


@jax.jit
def pallas_sequential_preLN__spectral_gfnet__glu_gated_bilinear__prompt_kernel(
    A_x, A_w_r, A_w_i, B_x, B_w_gate, B_w_up, B_w_down,
):
    del B_x
    xT = jnp.transpose(A_x.reshape(S, D))
    any_spec = pl.BlockSpec(memory_space=pl.ANY)
    vm = pltpu.VMEM
    dma = pltpu.SemaphoreType.DMA
    slab = vm((2 * PY * N1, 128), BF)
    oT = pl.pallas_call(
        _kernel,
        out_shape=jax.ShapeDtypeStruct((D, S), BF),
        in_specs=[any_spec] * 10,
        out_specs=any_spec,
        scratch_shapes=[
            vm((D, S), BF), vm((H + 1, S), BF), vm((H + 1, S), BF),
            vm((D, FF), BF), vm((D, FF), BF), vm((D, FF), BF),
            vm(_RF.shape, BF), vm(_CI.shape, BF), vm(_FA.shape, BF), vm(_GT.shape, F32),
            vm((N1, 128, 128), BF), vm((N1, 2, 128, 128), F32),
            vm((2, D, 128), F32), vm((NT, D, 128), BF), vm((NT, 2, 256, 128), BF),
            vm((N1 * PZ, 128), U32), vm((N1 * PZ, 128), U32),
            slab, slab, slab, slab,
            vm((N2 * PW, 128), U32), vm((N2 * PW, 128), U32),
            slab, slab,
            vm((2, 4, D, 128), BF), vm((4, D, 128), F32),
            vm((49, 128, 128), BF), vm((7, 2, 2, 128, 128), BF),
            vm((NC2, 49, Q, 128), BF), vm((NC2, 49, Q, 128), BF),
            vm((7, 2, Q, 128), BF), vm((7, 2, Q, 128), BF),
            vm((7, NKT, H, 128), BF), vm((7, NKT, 256, 128), BF), vm((D, S), BF),
            dma((NXC,)), dma((13,)), dma((NB + 2,)), pltpu.SemaphoreType.REGULAR,
        ],
        compiler_params=pltpu.CompilerParams(vmem_limit_bytes=100 * 1024 * 1024),
        name="gfnet_glu",
    )(xT, A_w_r.T, A_w_i.T, B_w_gate, B_w_up, B_w_down.T, _RF, _CI, _FA, _GT)
    return jnp.transpose(oT).reshape(1, S, D)
```
